```python
import os as _os
_os.environ.setdefault("JAX_PLATFORMS", "cpu")
import jax
import jax.numpy as jnp

def _softmax(x, axis=-1):
    return jax.nn.softmax(x, axis=axis)
def _gelu(x):
    return jax.nn.gelu(x, approximate=True)
def _silu(x):
    return jax.nn.silu(x)
def _sigmoid(x):
    return jax.nn.sigmoid(x)
def _layernorm(x, axis=-1, eps=1e-5):
    m = jnp.mean(x, axis=axis, keepdims=True)
    v = jnp.var(x, axis=axis, keepdims=True)
    return (x - m) / jnp.sqrt(v + eps)
def _scatter_add(tgt, idx, src, axis=0):
    return tgt.at[idx].add(src)
def _segment_sum(src, seg, n):
    return jax.ops.segment_sum(src, seg, n)
class _Rng:
    def __init__(self, key):
        self._k = key
    def _next(self):
        self._k, sub = jax.random.split(self._k)
        return sub
    def normal(self, shape):
        return jax.random.normal(self._next(), shape, dtype=jnp.bfloat16)
    def randint(self, lo, hi, shape):
        return jax.random.randint(self._next(), shape, lo, hi, dtype=jnp.int32)
    def uniform(self, shape, lo=0.0, hi=1.0):
        return jax.random.uniform(self._next(), shape, jnp.bfloat16, lo, hi)
    def permutation(self, n):
        return jax.random.permutation(self._next(), n)


kernel_name = 'gated_mix__linear_attn_block__glu_gated_swiglu__prompt'

def setup_inputs():
    _rng = _Rng(jax.random.key(int.from_bytes(__import__("os").urandom(4), "little")))
    _w = (lambda a: (lambda t: t.astype(jnp.bfloat16) if jnp.issubdtype(t.dtype, jnp.floating) else t)(jnp.asarray(a)))
    def _A_setup():
        B, S, D = 1, 2048, 1024
        return {
            "x": _w((lambda *s: _rng.normal(s) * 0.05)(B, S, D)),
            "wqkv": _w((lambda *s: _rng.normal(s) * 0.8)(D, 3 * D)),
            "wo": _w((lambda *s: _rng.normal(s) * 0.05)(D, D)),
        }
    _A_in = _A_setup()

    def _B_setup():
        B, S, D, F = 1, 2048, 1024, 3584
        return {
            "x": _w((lambda *s: _rng.normal(s) * 0.05)(B, S, D)),
            "w1": _w((lambda *s: _rng.normal(s) * 1.6)(D, F) * (2.0 / D) ** 0.5),
            "w3": _w((lambda *s: _rng.normal(s) * 1.6)(D, F) * (2.0 / D) ** 0.5),
            "w2": _w((lambda *s: _rng.normal(s) * 1.6)(F, D) * (2.0 / F) ** 0.5),
        }
    _B_in = _B_setup()

    return {
        "A_x": _A_in["x"],
        "A_wqkv": _A_in["wqkv"],
        "A_wo": _A_in["wo"],
        "B_x": _B_in["x"],
        "B_w1": _B_in["w1"],
        "B_w3": _B_in["w3"],
        "B_w2": _B_in["w2"],
        "gate_w": _w((lambda *s: _rng.normal(s) * 0.05)(1024) * 16.0),
    }

def reference(A_x, A_wqkv, A_wo, B_x, B_w1, B_w3, B_w2, gate_w):
    def _A_ref(x, wqkv, wo):
        B, S, D = x.shape
        H = 32; Dh = D // H
        qkv = (lambda x, *d: x.transpose(*d))((x @ wqkv).reshape(B, S, 3, H, Dh), 2, 0, 3, 1, 4)
        q, k, v = qkv[0], qkv[1], qkv[2]
        phi = lambda t: jnp.where(t > 0, t + 1, jnp.exp(t)) + 1e-6
        pq, pk = phi(q), phi(k)
        kv = jnp.einsum("bhsd,bhse->bhde", pk, v)
        z = jnp.einsum("bhsd->bhd", pk)
        num = jnp.einsum("bhqd,bhde->bhqe", pq, kv)
        den = jnp.einsum("bhqd,bhd->bhq", pq, z)[..., None] + 1e-6
        o = num / den
        return (lambda x, *d: x.transpose(*d))(o, 0, 2, 1, 3).reshape(B, S, D) @ wo

    def _B_ref(x, w1, w3, w2):
        gate = jnp.einsum("bsd,df->bsf", x, w1)
        up = jnp.einsum("bsd,df->bsf", x, w3)
        h = _silu(gate) * up
        out = jnp.einsum("bsf,fd->bsd", h, w2)
        return out

    x = A_x
    g = _sigmoid((x * gate_w).sum(-1, keepdims=True))
    a = _A_ref(x, A_wqkv, A_wo)
    b = _B_ref(x, B_w1, B_w3, B_w2)
    return g * a + (1 - g) * b
```

```python
import functools
import jax
import jax.numpy as jnp
import numpy as np
from jax import lax
from jax.experimental import pallas as pl
from jax.experimental.pallas import tpu as pltpu

BF = jnp.bfloat16
F32 = jnp.float32


def _phi(t):
    return jnp.where(t > 0, t + 1.0, jnp.exp(t)) + 1e-6


def _dot(a, b):
    return jnp.dot(a, b, preferred_element_type=F32)


def make(tm1=512, tm2=512, fc=512, vmem_mb=100):
    S, D, F, H = 2048, 1024, 3584, 32
    DH = D // H
    G = D // 128
    n1 = S // tm1
    n2 = S // tm2
    nf = F // fc

    def kernel(x_hbm, wqkv_hbm, wo_hbm, w1_hbm, w3_hbm, w2_hbm, gw_ref, o_hbm,
               x_v, wqkv_v, wo_v, w1_v, w3_v, w2_v, o_v, kv_acc, z_acc, m_v, zm_v, h_v, sems):
        copies = []
        def mk(src, dst):
            c = pltpu.make_async_copy(src, dst, sems.at[len(copies)])
            copies.append(c)
            return c
        cx = [mk(x_hbm.at[pl.ds(i * tm1, tm1)], x_v.at[pl.ds(i * tm1, tm1)]) for i in range(1)]
        ck = mk(wqkv_hbm.at[:, pl.ds(D, D)], wqkv_v.at[:, pl.ds(D, D)])
        cv = mk(wqkv_hbm.at[:, pl.ds(2 * D, D)], wqkv_v.at[:, pl.ds(2 * D, D)])
        cx += [mk(x_hbm.at[pl.ds(i * tm1, tm1)], x_v.at[pl.ds(i * tm1, tm1)]) for i in range(1, n1)]
        cwo = mk(wo_hbm, wo_v)
        cq = mk(wqkv_hbm.at[:, pl.ds(0, D)], wqkv_v.at[:, pl.ds(0, D)])
        c1 = mk(w1_hbm, w1_v)
        c3 = mk(w3_hbm, w3_v)
        c2 = mk(w2_hbm, w2_v)
        for c in copies:
            c.start()

        kv_acc[...] = jnp.zeros_like(kv_acc)
        z_acc[...] = jnp.zeros_like(z_acc)
        ck.wait()
        cv.wait()

        def p1(i, c):
            r0 = pl.multiple_of(i * tm1, tm1)
            pltpu.make_async_copy(x_hbm.at[pl.ds(r0, tm1)], x_v.at[pl.ds(r0, tm1)],
                                  sems.at[jnp.where(i == 0, 0, i + 2)]).wait()
            xi = x_v[pl.ds(r0, tm1), :]
            k = _dot(xi, wqkv_v[:, D:2 * D])
            pk = _phi(k)
            z_acc[...] += jnp.sum(pk.reshape(tm1 // 8, 8, D), axis=0)
            pkb = pk.astype(BF)
            vb = _dot(xi, wqkv_v[:, 2 * D:3 * D]).astype(BF)
            for g in range(G):
                kv_acc[g] += lax.dot_general(pkb[:, g * 128:(g + 1) * 128], vb[:, g * 128:(g + 1) * 128],
                                             (((0,), (0,)), ((), ())), preferred_element_type=F32)
            return c
        lax.fori_loop(0, n1, p1, 0)

        cwo.wait()
        ri = lax.broadcasted_iota(jnp.int32, (128, 128), 0) // DH
        ci = lax.broadcasted_iota(jnp.int32, (128, 128), 1) // DH
        same = ri == ci
        z = jnp.sum(z_acc[...], axis=0, keepdims=True)
        for g in range(G):
            kvg = jnp.where(same, kv_acc[g], 0.0).astype(BF)
            m_v[g * 128:(g + 1) * 128, :] = _dot(kvg, wo_v[g * 128:(g + 1) * 128, :]).astype(BF)
            zg = jnp.broadcast_to(z[:, g * 128:(g + 1) * 128], (128, 128))
            zm_v[g] = jnp.where(same, zg, 0.0).astype(BF)

        cq.wait()
        c1.wait()
        c3.wait()
        c2.wait()

        def p2(i, c):
            r0 = pl.multiple_of(i * tm2, tm2)
            xi = x_v[pl.ds(r0, tm2), :]
            gate = jax.nn.sigmoid(jnp.sum(xi.astype(F32) * gw_ref[...].astype(F32), axis=-1, keepdims=True))
            q = _dot(xi, wqkv_v[:, 0:D])
            pq = _phi(q)
            pqb = pq.astype(BF)
            parts = []
            for g in range(G):
                den = lax.dot_general(pqb[:, g * 128:(g + 1) * 128], zm_v[g], (((1,), (1,)), ((), ())),
                                      preferred_element_type=F32) + 1e-6
                parts.append((pq[:, g * 128:(g + 1) * 128] * (gate / den)).astype(BF))
            pqn = jnp.concatenate(parts, axis=1)
            a = _dot(pqn, m_v[...])
            for j in range(nf):
                gt = _dot(xi, w1_v[:, j * fc:(j + 1) * fc])
                up = _dot(xi, w3_v[:, j * fc:(j + 1) * fc])
                h_v[:, j * fc:(j + 1) * fc] = (gt * jax.nn.sigmoid(gt) * up).astype(BF)
            b = _dot(h_v[...], w2_v[...])
            o_v[pl.ds(r0, tm2), :] = (a + (1.0 - gate) * b).astype(BF)
            pltpu.make_async_copy(o_v.at[pl.ds(r0, tm2)], o_hbm.at[pl.ds(r0, tm2)], osem.at[i]).start()
            return c
        osem = sems.at[pl.ds(len(copies), n2)]
        lax.fori_loop(0, n2, p2, 0)
        for i in range(n2):
            pltpu.make_async_copy(o_v.at[pl.ds(i * tm2, tm2)], o_hbm.at[pl.ds(i * tm2, tm2)], osem.at[i]).wait()

    nsem = n1 + 8 + n2

    def fn(A_x, A_wqkv, A_wo, B_x, B_w1, B_w3, B_w2, gate_w):
        x = A_x.reshape(S, D)
        gw = gate_w.reshape(1, D)
        anyspec = pl.BlockSpec(memory_space=pl.ANY)
        out = pl.pallas_call(
            kernel,
            in_specs=[anyspec] * 6 + [pl.BlockSpec((1, D), lambda: (0, 0))],
            out_specs=anyspec,
            out_shape=jax.ShapeDtypeStruct((S, D), BF),
            scratch_shapes=[
                pltpu.VMEM((S, D), BF),
                pltpu.VMEM((D, 3 * D), BF),
                pltpu.VMEM((D, D), BF),
                pltpu.VMEM((D, F), BF),
                pltpu.VMEM((D, F), BF),
                pltpu.VMEM((F, D), BF),
                pltpu.VMEM((S, D), BF),
                pltpu.VMEM((G, 128, 128), F32),
                pltpu.VMEM((8, D), F32),
                pltpu.VMEM((D, D), BF),
                pltpu.VMEM((G, 128, 128), BF),
                pltpu.VMEM((tm2, F), BF),
                pltpu.SemaphoreType.DMA((nsem,)),
            ],
            compiler_params=pltpu.CompilerParams(vmem_limit_bytes=vmem_mb * 1024 * 1024),
        )(x, A_wqkv, A_wo, B_w1, B_w3, B_w2, gw)
        return out.reshape(1, S, D)
    return fn


_impl = make(512, 512, 512)


@jax.jit
def pallas_gated_mix__linear_attn_block__glu_gated_swiglu__prompt_kernel(
    A_x: jax.Array,
    A_wqkv: jax.Array,
    A_wo: jax.Array,
    B_x: jax.Array,
    B_w1: jax.Array,
    B_w3: jax.Array,
    B_w2: jax.Array,
    gate_w: jax.Array,
):
    return _impl(A_x, A_wqkv, A_wo, B_x, B_w1, B_w3, B_w2, gate_w)
```

```python
import contextlib
import jax
import jax.numpy as jnp
import numpy as np
from jax import lax
from jax.experimental import pallas as pl
from jax.experimental.pallas import tpu as pltpu

BF = jnp.bfloat16
F32 = jnp.float32


def _phi(t):
    return jnp.where(t > 0, t + 1.0, jnp.exp(t)) + 1e-6


def _dot(a, b):
    return jnp.dot(a, b, preferred_element_type=F32)


def make(r0=512, tm1=512, tm2=128, fc=512,
         plan=(256, 512, 1024), lcuts=(1024,), defer='next',
         vmem_mb=100, scopes=False, norm_at=2, silu='approx', osplit=1):
    S, D, F, H = 2048, 1024, 3584, 32
    DH = D // H
    G = D // 128
    n1 = (S - r0) // tm1
    assert r0 + n1 * tm1 == S
    n2 = S // tm2
    nf = F // fc
    scope = (lambda n: jax.named_scope(n)) if scopes else (lambda n: contextlib.nullcontext())
    base = {'k': D, 'v': 2 * D}
    pc = [0] + list(plan)
    lc = [0] + list(lcuts)
    nchunks = len(plan)
    nsem = 1 + nchunks + n1 + 1 + 1

    def kernel(x_hbm, wqkv_hbm, wo_hbm, w1_hbm, w3_hbm, w2_hbm, gw_hbm, o_hbm,
               x_v, wqkv_v, wo_v, w1_v, w3_v, w2_v, gw_v, o_v, kx_acc, z_acc, m_v, h_v, pqn_v, zr_v,
               sems):
        ctr = [0]
        def mk(src, dst):
            c = pltpu.make_async_copy(src, dst, sems.at[ctr[0]])
            ctr[0] += 1
            return c
        def cols(ref, a, b):
            return ref.at[:, pl.ds(a, b - a)]
        cx0 = mk(x_hbm.at[pl.ds(0, r0)], x_v.at[pl.ds(0, r0)])
        cst = [mk(cols(wqkv_hbm, D + pc[c], D + pc[c + 1]), cols(wqkv_v, D + pc[c], D + pc[c + 1]))
               for c in range(nchunks)]
        xbase = ctr[0]
        cx = [mk(x_hbm.at[pl.ds(r0 + i * tm1, tm1)], x_v.at[pl.ds(r0 + i * tm1, tm1)]) for i in range(n1)]
        rsem = sems.at[ctr[0]]
        crest = [pltpu.make_async_copy(a_, b_, rsem) for (a_, b_) in (
            (gw_hbm, gw_v), (cols(wqkv_hbm, 2 * D, 3 * D), cols(wqkv_v, 2 * D, 3 * D)), (wo_hbm, wo_v),
            (cols(wqkv_hbm, 0, D), cols(wqkv_v, 0, D)), (w1_hbm, w1_v), (w3_hbm, w3_v), (w2_hbm, w2_v))]
        obase = ctr[0] + 1
        for c in [cx0] + cst + cx + crest:
            c.start()

        def k_part(xi, a, b, first):
            pk = _phi(_dot(xi, wqkv_v[:, D + a:D + b]))
            zs = jnp.sum(pk.reshape(pk.shape[0] // 8, 8, b - a), axis=0)
            if first:
                z_acc[:, a:b] = zs
            else:
                z_acc[:, a:b] += zs
            return pk.astype(BF)

        def kx_part(xi, pkb, a, b, first):
            kx = lax.dot_general(pkb, xi, (((0,), (0,)), ((), ())), preferred_element_type=F32)
            if first:
                kx_acc[a:b, :] = kx
            else:
                kx_acc[a:b, :] += kx

        with scope("p1_first"):
            prev = []
            for c in range(nchunks):
                with scope("w%d" % c):
                    if c == 0:
                        cx0.wait()
                    cst[c].wait()
                xi = x_v[0:r0, :]
                cur = (k_part(xi, pc[c], pc[c + 1], True), pc[c], pc[c + 1])
                if defer == 'next':
                    for (pkb, a, b) in prev:
                        kx_part(xi, pkb, a, b, True)
                    prev = [cur]
                elif defer == 'end':
                    prev.append(cur)
                else:
                    kx_part(xi, *cur, True)
            for (pkb, a, b) in prev:
                kx_part(xi, pkb, a, b, True)

        def p1(i, carry):
            rr = pl.multiple_of(r0 + i * tm1, 16)
            pltpu.make_async_copy(x_hbm.at[pl.ds(rr, tm1)], x_v.at[pl.ds(rr, tm1)], sems.at[xbase + i]).wait()
            xi = x_v[pl.ds(rr, tm1), :]
            pend = []
            for c in range(len(lcuts)):
                cur = (k_part(xi, lc[c], lc[c + 1], False), lc[c], lc[c + 1])
                for (pkb, a, b) in pend:
                    kx_part(xi, pkb, a, b, False)
                pend = [cur]
            for (pkb, a, b) in pend:
                kx_part(xi, pkb, a, b, False)
            return carry
        with scope("p1_rest"):
            lax.fori_loop(0, n1, p1, 0)

        with scope("wait_ffn"):
            for c in crest:
                c.wait()
        with scope("mid"):
            ri = lax.broadcasted_iota(jnp.int32, (128, 128), 0) // DH
            ci = lax.broadcasted_iota(jnp.int32, (128, 128), 1) // DH
            same = ri == ci
            zr_v[...] = jnp.sum(z_acc[...], axis=0, keepdims=True)
            kvs = []
            for g in range(G):
                kvg = _dot(kx_acc[g * 128:(g + 1) * 128, :].astype(BF), wqkv_v[:, 2 * D + g * 128:2 * D + (g + 1) * 128])
                kvs.append(jnp.where(same, kvg, 0.0).astype(BF))
            for g in range(G):
                m_v[g * 128:(g + 1) * 128, :] = _dot(kvs[g], wo_v[g * 128:(g + 1) * 128, :]).astype(BF)

        oc = D // osplit
        def o_copy(rr, i, s):
            return pltpu.make_async_copy(o_v.at[pl.ds(rr, tm2), pl.ds(s * oc, oc)],
                                         o_hbm.at[pl.ds(rr, tm2), pl.ds(s * oc, oc)], sems.at[obase])

        def p2(i, carry):
            rr = pl.multiple_of(i * tm2, tm2)
            xi = x_v[pl.ds(rr, tm2), :]
            gate = jax.nn.sigmoid(jnp.sum(xi.astype(F32) * gw_v[...].astype(F32).reshape(1, D), axis=-1, keepdims=True))
            pq = _phi(_dot(xi, wqkv_v[:, 0:D]))

            def ffn_chunk(j):
                gt = _dot(xi, w1_v[:, j * fc:(j + 1) * fc])
                up = _dot(xi, w3_v[:, j * fc:(j + 1) * fc])
                if silu == 'exact':
                    hh = gt * jax.nn.sigmoid(gt) * up
                else:
                    hh = gt * pltpu.reciprocal(1.0 + jnp.exp(-gt), approx=True) * up
                h_v[:, j * fc:(j + 1) * fc] = hh.astype(BF)

            def vpu_norm():
                lane = lax.broadcasted_iota(jnp.int32, (tm2, 128), 1)
                zrow = zr_v[...]
                def swap(y, s):
                    return jnp.take_along_axis(y, lane ^ s, axis=1)
                cur = [pq[:, g * 128:(g + 1) * 128] * zrow[:, g * 128:(g + 1) * 128] for g in range(G)]
                for s in (16, 8, 4):
                    m = (lane & s) == 0
                    n = len(cur) // 2
                    cur = [jnp.where(m, cur[t], cur[t + n]) + swap(jnp.where(m, cur[t + n], cur[t]), s)
                           for t in range(n)]
                y = cur[0]
                for s in (2, 1):
                    y = y + swap(y, s)
                r = gate * pltpu.reciprocal(y + 1e-6, approx=True)
                for g in range(G):
                    rg = jnp.take_along_axis(r, (lane & 96) + 4 * g, axis=1)
                    sl = slice(g * 128, (g + 1) * 128)
                    pqn_v[:, sl] = (pq[:, sl] * rg).astype(BF)

            for j in range(nf):
                ffn_chunk(j)
                if j + 1 == norm_at:
                    vpu_norm()
            for s in range(osplit):
                cs = slice(s * oc, (s + 1) * oc)
                b = _dot(h_v[...], w2_v[:, cs])
                o = (1.0 - gate) * b + _dot(pqn_v[...], m_v[:, cs])
                o_v[pl.ds(rr, tm2), cs] = o.astype(BF)
                o_copy(rr, i, s).start()
            return carry
        with scope("phase2"):
            lax.fori_loop(0, n2, p2, 0)
        with scope("tail"):
            pltpu.make_async_copy(o_v, o_hbm, sems.at[obase]).wait()

    def fn(A_x, A_wqkv, A_wo, B_x, B_w1, B_w3, B_w2, gate_w):
        x = A_x.reshape(S, D)
        anyspec = pl.BlockSpec(memory_space=pl.ANY)
        out = pl.pallas_call(
            kernel,
            in_specs=[anyspec] * 7,
            out_specs=anyspec,
            out_shape=jax.ShapeDtypeStruct((S, D), BF),
            scratch_shapes=[
                pltpu.VMEM((S, D), BF),
                pltpu.VMEM((D, 3 * D), BF),
                pltpu.VMEM((D, D), BF),
                pltpu.VMEM((D, F), BF),
                pltpu.VMEM((D, F), BF),
                pltpu.VMEM((F, D), BF),
                pltpu.VMEM((D,), BF),
                pltpu.VMEM((S, D), BF),
                pltpu.VMEM((D, D), F32),
                pltpu.VMEM((8, D), F32),
                pltpu.VMEM((D, D), BF),
                pltpu.VMEM((tm2, F), BF),
                pltpu.VMEM((tm2, D), BF),
                pltpu.VMEM((1, D), F32),
                pltpu.SemaphoreType.DMA((nsem,)),
            ],
            compiler_params=pltpu.CompilerParams(vmem_limit_bytes=vmem_mb * 1024 * 1024),
        )(x, A_wqkv, A_wo, B_w1, B_w3, B_w2, gate_w)
        return out.reshape(1, S, D)
    return fn


_impl = make(r0=128, tm1=384, tm2=256, osplit=4, plan=(256, 512, 768, 1024))


@jax.jit
def pallas_gated_mix__linear_attn_block__glu_gated_swiglu__prompt_kernel(
    A_x: jax.Array,
    A_wqkv: jax.Array,
    A_wo: jax.Array,
    B_x: jax.Array,
    B_w1: jax.Array,
    B_w3: jax.Array,
    B_w2: jax.Array,
    gate_w: jax.Array,
):
    return _impl(A_x, A_wqkv, A_wo, B_x, B_w1, B_w3, B_w2, gate_w)
```

```python
import contextlib
import jax
import jax.numpy as jnp
import numpy as np
from jax import lax
from jax.experimental import pallas as pl
from jax.experimental.pallas import tpu as pltpu

BF = jnp.bfloat16
F32 = jnp.float32


def _phi(t):
    return jnp.where(t > 0, t + 1.0, jnp.exp(t)) + 1e-6


def _dot(a, b):
    return jnp.dot(a, b, preferred_element_type=F32)


def make(r0=512, tm1=512, tm2=128, fc=512,
         plan=(256, 512, 1024), lcuts=(1024,), defer='next', strassen=True, fs=256, order=(1, 4, 5, 7, 2, 3, 6), pcols=512, packed=False,
         vmem_mb=100, scopes=False, norm_at=2, silu='approx', osplit=1):
    S, D, F, H = 2048, 1024, 3584, 32
    DH = D // H
    G = D // 128
    n1 = (S - r0) // tm1
    assert r0 + n1 * tm1 == S
    n2 = S // tm2
    nf = F // fc
    scope = (lambda n: jax.named_scope(n)) if scopes else (lambda n: contextlib.nullcontext())
    base = {'k': D, 'v': 2 * D}
    pc = [0] + list(plan)
    lc = [0] + list(lcuts)
    nchunks = len(plan)
    nsem = 1 + nchunks + n1 + 1 + 1

    def kernel(x_hbm, wqkv_hbm, wo_hbm, w1_hbm, w3_hbm, w2_hbm, gw_hbm, o_hbm,
               x_v, wqkv_v, wo_v, w1_v, w3_v, w2_v, gw_v, o_v, kx_acc, z_acc, m_v, bu_v, bd_v, ad_v, pqn_v, zr_v,
               sems):
        ctr = [0]
        def mk(src, dst):
            c = pltpu.make_async_copy(src, dst, sems.at[ctr[0]])
            ctr[0] += 1
            return c
        def cols(ref, a, b):
            return ref.at[:, pl.ds(a, b - a)]
        cx0 = mk(x_hbm.at[pl.ds(0, r0)], x_v.at[pl.ds(0, r0)])
        cst = [mk(cols(wqkv_hbm, D + pc[c], D + pc[c + 1]), cols(wqkv_v, D + pc[c], D + pc[c + 1]))
               for c in range(nchunks)]
        xbase = ctr[0]
        cx = [mk(x_hbm.at[pl.ds(r0 + i * tm1, tm1)], x_v.at[pl.ds(r0 + i * tm1, tm1)]) for i in range(n1)]
        rsem = sems.at[ctr[0]]
        crest = [pltpu.make_async_copy(a_, b_, rsem) for (a_, b_) in (
            (gw_hbm, gw_v), (cols(wqkv_hbm, 2 * D, 3 * D), cols(wqkv_v, 2 * D, 3 * D)), (wo_hbm, wo_v),
            (cols(wqkv_hbm, 0, D), cols(wqkv_v, 0, D)), (w1_hbm, w1_v), (w3_hbm, w3_v), (w2_hbm, w2_v))]
        obase = ctr[0] + 1
        for c in [cx0] + cst + cx + crest:
            c.start()

        def k_part(xi, a, b, first):
            pk = _phi(_dot(xi, wqkv_v[:, D + a:D + b]))
            zs = jnp.sum(pk.reshape(pk.shape[0] // 8, 8, b - a), axis=0)
            if first:
                z_acc[:, a:b] = zs
            else:
                z_acc[:, a:b] += zs
            return pk.astype(BF)

        def kx_part(xi, pkb, a, b, first):
            kx = lax.dot_general(pkb, xi, (((0,), (0,)), ((), ())), preferred_element_type=F32)
            if first:
                kx_acc[a:b, :] = kx
            else:
                kx_acc[a:b, :] += kx

        with scope("p1_first"):
            prev = []
            for c in range(nchunks):
                with scope("w%d" % c):
                    if c == 0:
                        cx0.wait()
                    cst[c].wait()
                xi = x_v[0:r0, :]
                cur = (k_part(xi, pc[c], pc[c + 1], True), pc[c], pc[c + 1])
                if defer == 'next':
                    for (pkb, a, b) in prev:
                        kx_part(xi, pkb, a, b, True)
                    prev = [cur]
                elif defer == 'end':
                    prev.append(cur)
                else:
                    kx_part(xi, *cur, True)
            for (pkb, a, b) in prev:
                kx_part(xi, pkb, a, b, True)

        def p1(i, carry):
            rr = pl.multiple_of(r0 + i * tm1, 16)
            pltpu.make_async_copy(x_hbm.at[pl.ds(rr, tm1)], x_v.at[pl.ds(rr, tm1)], sems.at[xbase + i]).wait()
            xi = x_v[pl.ds(rr, tm1), :]
            pend = []
            for c in range(len(lcuts)):
                cur = (k_part(xi, lc[c], lc[c + 1], False), lc[c], lc[c + 1])
                for (pkb, a, b) in pend:
                    kx_part(xi, pkb, a, b, False)
                pend = [cur]
            for (pkb, a, b) in pend:
                kx_part(xi, pkb, a, b, False)
            return carry
        with scope("p1_rest"):
            lax.fori_loop(0, n1, p1, 0)

        with scope("wait_ffn"):
            for c in crest:
                c.wait()
        with scope("mid"):
            ri = lax.broadcasted_iota(jnp.int32, (128, 128), 0) // DH
            ci = lax.broadcasted_iota(jnp.int32, (128, 128), 1) // DH
            same = ri == ci
            zr_v[...] = jnp.sum(z_acc[...], axis=0, keepdims=True)
            kvs = []
            for g in range(G):
                kvg = _dot(kx_acc[g * 128:(g + 1) * 128, :].astype(BF), wqkv_v[:, 2 * D + g * 128:2 * D + (g + 1) * 128])
                kvs.append(jnp.where(same, kvg, 0.0).astype(BF))
            for g in range(G):
                m_v[g * 128:(g + 1) * 128, :] = _dot(kvs[g], wo_v[g * 128:(g + 1) * 128, :]).astype(BF)

        def pk(v):
            return pltpu.bitcast(v, jnp.uint32)
        def upk(v):
            return pltpu.bitcast(v, BF)

        def combos(b11, b12, b21, b22):
            f11, f12, f21, f22 = (t.astype(F32) for t in (b11, b12, b21, b22))
            return [(f11 + f22).astype(BF), (f12 - f22).astype(BF), (f21 - f11).astype(BF),
                    (f11 + f12).astype(BF), (f21 + f22).astype(BF)]

        def st(ref, n, r, nr, cs, val):
            if packed:
                ref[n, pl.ds(pl.multiple_of(r // 2, 8), nr // 2), cs] = pk(val)
            else:
                ref[n, pl.ds(r, nr), cs] = val
        def ld(ref, n, cs):
            return upk(ref[n, :, cs]) if packed else ref[n, :, cs]

        cidx = (0, None, 1, 2, None, 3, 4)
        def b_up(n, c0, c1):
            if n == 1:
                return w1_v[0:D // 2, c0:c1]
            if n == 4:
                return w3_v[D // 2:D, c0:c1]
            return ld(bu_v, cidx[n], slice(c0, c1))
        def b_dn(n, c0, c1):
            if n == 1:
                return w2_v[0:F // 2, c0:c1]
            if n == 4:
                return w2_v[F // 2:F, D // 2 + c0:D // 2 + c1]
            return ld(bd_v, cidx[n], slice(c0, c1))

        def pre_up(t, c):
            r = pl.multiple_of(t * 16, 16)
            for c0 in range(0, F, pcols):
                cs = slice(c0, c0 + pcols)
                out = combos(w1_v[pl.ds(r, 16), cs], w3_v[pl.ds(r, 16), cs],
                             w1_v[pl.ds(D // 2 + r, 16), cs], w3_v[pl.ds(D // 2 + r, 16), cs])
                for n in range(5):
                    st(bu_v, n, r, 16, cs, out[n])
            return c
        def pre_dn(t, c):
            r = pl.multiple_of(t * 64, 64)
            for r1 in range(0, 64, 16):
                out = combos(w2_v[pl.ds(r + r1, 16), 0:D // 2], w2_v[pl.ds(r + r1, 16), D // 2:D],
                             w2_v[pl.ds(F // 2 + r + r1, 16), 0:D // 2], w2_v[pl.ds(F // 2 + r + r1, 16), D // 2:D])
                for n in range(5):
                    st(bd_v, n, r + r1, 16, slice(None), out[n])
            return c
        with scope("pre"):
            lax.fori_loop(0, (D // 2) // 16, pre_up, 0)
            lax.fori_loop(0, (F // 2) // 64, pre_dn, 0)

        oc = D // osplit
        hm = tm2 // 2
        def o_copy(rr, i, s):
            return pltpu.make_async_copy(o_v.at[pl.ds(rr, tm2), pl.ds(s * oc, oc)],
                                         o_hbm.at[pl.ds(rr, tm2), pl.ds(s * oc, oc)], sems.at[obase])

        def a_combos(a11, a12, a21, a22):
            return [a11 + a22, a21 + a22, a11, a22, a11 + a12, a21 - a11, a12 - a22]

        def strassen_c(prod):
            m = {}
            def g(n):
                if n not in m:
                    m[n] = prod(n - 1)
                return m[n]
            for n in order:
                g(n)
            c11 = g(1) + g(4) - g(5) + g(7)
            c12 = g(3) + g(5)
            c21 = g(2) + g(4)
            c22 = g(1) - g(2) + g(3) + g(6)
            return c11, c12, c21, c22

        def p2(i, carry):
            rr = pl.multiple_of(i * tm2, tm2)
            xi = x_v[pl.ds(rr, tm2), :]
            gate = jax.nn.sigmoid(jnp.sum(xi.astype(F32) * gw_v[...].astype(F32).reshape(1, D), axis=-1, keepdims=True))
            pq = _phi(_dot(xi, wqkv_v[:, 0:D]))
            xf = xi.astype(F32)
            au = [t.astype(BF) for t in a_combos(xf[0:hm, 0:D // 2], xf[0:hm, D // 2:D], xf[hm:tm2, 0:D // 2], xf[hm:tm2, D // 2:D])]

            def hchunk(c0, c1):
                c11, c12, c21, c22 = strassen_c(lambda n: _dot(au[n], b_up(n, c0, c1)))
                def act(gt, up):
                    if silu == 'exact':
                        return gt * jax.nn.sigmoid(gt) * up
                    return gt * pltpu.reciprocal(1.0 + jnp.exp(-gt), approx=True) * up
                return act(c11, c12), act(c21, c22)

            def vpu_norm():
                lane = lax.broadcasted_iota(jnp.int32, (tm2, 128), 1)
                zrow = zr_v[...]
                def swap(y, s):
                    return jnp.take_along_axis(y, lane ^ s, axis=1)
                cur = [pq[:, g * 128:(g + 1) * 128] * zrow[:, g * 128:(g + 1) * 128] for g in range(G)]
                for s in (16, 8, 4):
                    m = (lane & s) == 0
                    n = len(cur) // 2
                    cur = [jnp.where(m, cur[t], cur[t + n]) + swap(jnp.where(m, cur[t + n], cur[t]), s)
                           for t in range(n)]
                y = cur[0]
                for s in (2, 1):
                    y = y + swap(y, s)
                r = gate * pltpu.reciprocal(y + 1e-6, approx=True)
                for g in range(G):
                    rg = jnp.take_along_axis(r, (lane & 96) + 4 * g, axis=1)
                    sl = slice(g * 128, (g + 1) * 128)
                    pqn_v[:, sl] = (pq[:, sl] * rg).astype(BF)

            nfs = (F // 2) // fs
            for j in range(nfs):
                c0, c1 = j * fs, (j + 1) * fs
                a11, a21 = hchunk(c0, c1)
                a12, a22 = hchunk(F // 2 + c0, F // 2 + c1)
                for n, t in enumerate(a_combos(a11, a12, a21, a22)):
                    ad_v[n, :, c0:c1] = t.astype(BF)
                if j + 1 == norm_at:
                    vpu_norm()
            hw = D // 2
            for s in range(osplit // 2):
                c0, c1 = s * oc, (s + 1) * oc
                c11, c12, c21, c22 = strassen_c(lambda n: _dot(ad_v[n], b_dn(n, c0, c1)))
                for (ct, cb, off) in ((c11, c21, 0), (c12, c22, hw)):
                    cs = slice(off + c0, off + c1)
                    b = jnp.concatenate([ct, cb], axis=0)
                    o = (1.0 - gate) * b + _dot(pqn_v[...], m_v[:, cs])
                    o_v[pl.ds(rr, tm2), cs] = o.astype(BF)
                    o_copy(rr, i, (off + c0) // oc).start()
            return carry
        with scope("phase2"):
            lax.fori_loop(0, n2, p2, 0)
        with scope("tail"):
            pltpu.make_async_copy(o_v, o_hbm, sems.at[obase]).wait()

    def fn(A_x, A_wqkv, A_wo, B_x, B_w1, B_w3, B_w2, gate_w):
        x = A_x.reshape(S, D)
        anyspec = pl.BlockSpec(memory_space=pl.ANY)
        out = pl.pallas_call(
            kernel,
            in_specs=[anyspec] * 7,
            out_specs=anyspec,
            out_shape=jax.ShapeDtypeStruct((S, D), BF),
            scratch_shapes=[
                pltpu.VMEM((S, D), BF),
                pltpu.VMEM((D, 3 * D), BF),
                pltpu.VMEM((D, D), BF),
                pltpu.VMEM((D, F), BF),
                pltpu.VMEM((D, F), BF),
                pltpu.VMEM((F, D), BF),
                pltpu.VMEM((D,), BF),
                pltpu.VMEM((S, D), BF),
                pltpu.VMEM((D, D), F32),
                pltpu.VMEM((8, D), F32),
                pltpu.VMEM((D, D), BF),
                (pltpu.VMEM((5, D // 4, F), jnp.uint32) if packed else pltpu.VMEM((5, D // 2, F), BF)),
                (pltpu.VMEM((5, F // 4, D // 2), jnp.uint32) if packed else pltpu.VMEM((5, F // 2, D // 2), BF)),
                pltpu.VMEM((7, tm2 // 2, F // 2), BF),
                pltpu.VMEM((tm2, D), BF),
                pltpu.VMEM((1, D), F32),
                pltpu.SemaphoreType.DMA((nsem,)),
            ],
            compiler_params=pltpu.CompilerParams(vmem_limit_bytes=vmem_mb * 1024 * 1024),
        )(x, A_wqkv, A_wo, B_w1, B_w3, B_w2, gate_w)
        return out.reshape(1, S, D)
    return fn


_impl = make(r0=128, tm1=384, tm2=256, osplit=4, plan=(256, 512, 768, 1024), fs=256, packed=False)


@jax.jit
def pallas_gated_mix__linear_attn_block__glu_gated_swiglu__prompt_kernel(
    A_x: jax.Array,
    A_wqkv: jax.Array,
    A_wo: jax.Array,
    B_x: jax.Array,
    B_w1: jax.Array,
    B_w3: jax.Array,
    B_w2: jax.Array,
    gate_w: jax.Array,
):
    return _impl(A_x, A_wqkv, A_wo, B_x, B_w1, B_w3, B_w2, gate_w)
```

```python
import contextlib
import jax
import jax.numpy as jnp
import numpy as np
from jax import lax
from jax.experimental import pallas as pl
from jax.experimental.pallas import tpu as pltpu

BF = jnp.bfloat16
F32 = jnp.float32


def _phi(t):
    return jnp.where(t > 0, t + 1.0, jnp.exp(t)) + 1e-6


def _dot(a, b):
    return jnp.dot(a, b, preferred_element_type=F32)


def _a_combos(a11, a12, a21, a22):
    return [a11 + a22, a21 + a22, a11, a22, a11 + a12, a21 - a11, a12 - a22]


def _b_combos(b11, b12, b21, b22):
    return [b11 + b22, b11, b12 - b22, b21 - b11, b22, b11 + b12, b21 + b22]


def _c_combos(prod, order=(0, 3, 4, 6, 1, 2, 5)):
    m = {n: prod(n) for n in order}
    return (m[0] + m[3] - m[4] + m[6], m[2] + m[4], m[1] + m[3], m[0] - m[1] + m[2] + m[5])


def make(r0=128, tm1=384, tm2=256, fs=256, plan=(256, 512, 768, 1024),
         vmem_mb=120, scopes=False, norm_at=1, osplit=4, pcols=512, overlap=False):
    S, D, F, H = 2048, 1024, 3584, 32
    DH = D // H
    G = D // 128
    HD, HF = D // 2, F // 2
    WU = F + HD
    KD = HF + HD
    n1 = (S - r0) // tm1
    assert r0 + n1 * tm1 == S
    n2 = S // tm2
    hm = tm2 // 2
    scope = (lambda n: jax.named_scope(n)) if scopes else (lambda n: contextlib.nullcontext())
    pc = [0] + list(plan)
    nchunks = len(plan)
    nsem = 1 + nchunks + n1 + 2
    RAW = (1, 4)

    def kernel(x_hbm, wqkv_hbm, wo_hbm, w1_hbm, w3_hbm, w2_hbm, gw_hbm, o_hbm,
               x_v, wkv_v, wo_v, bu_v, su_v, bd_v, sd_v, gw_v, o_v, kx_acc, z_acc, ad_v, zr_v,
               sems):
        ctr = [0]
        def mk(src, dst):
            c = pltpu.make_async_copy(src, dst, sems.at[ctr[0]])
            ctr[0] += 1
            return c
        cx0 = mk(x_hbm.at[pl.ds(0, r0)], x_v.at[pl.ds(0, r0)])
        cst = [mk(wqkv_hbm.at[:, pl.ds(D + pc[c], pc[c + 1] - pc[c])], wkv_v.at[:, pl.ds(pc[c], pc[c + 1] - pc[c])])
               for c in range(nchunks)]
        xbase = ctr[0]
        cx = [mk(x_hbm.at[pl.ds(r0 + i * tm1, tm1)], x_v.at[pl.ds(r0 + i * tm1, tm1)]) for i in range(n1)]
        rsem = sems.at[ctr[0]]
        osem = sems.at[ctr[0] + 1]
        crest = [pltpu.make_async_copy(a_, b_, rsem) for (a_, b_) in (
            (gw_hbm, gw_v),
            (wqkv_hbm.at[:, pl.ds(2 * D, D)], wkv_v.at[:, pl.ds(D, D)]),
            (wo_hbm, wo_v),
            (wqkv_hbm.at[pl.ds(0, HD), pl.ds(0, HD)], bu_v.at[1, :, pl.ds(F, HD)]),
            (wqkv_hbm.at[pl.ds(HD, HD), pl.ds(0, HD)], su_v.at[1, :, pl.ds(F, HD)]),
            (wqkv_hbm.at[pl.ds(0, HD), pl.ds(HD, HD)], su_v.at[0, :, pl.ds(F, HD)]),
            (wqkv_hbm.at[pl.ds(HD, HD), pl.ds(HD, HD)], bu_v.at[4, :, pl.ds(F, HD)]),
            (w1_hbm.at[pl.ds(0, HD)], bu_v.at[1, :, pl.ds(0, F)]),
            (w1_hbm.at[pl.ds(HD, HD)], su_v.at[1, :, pl.ds(0, F)]),
            (w3_hbm.at[pl.ds(0, HD)], su_v.at[0, :, pl.ds(0, F)]),
            (w3_hbm.at[pl.ds(HD, HD)], bu_v.at[4, :, pl.ds(0, F)]),
            (w2_hbm.at[pl.ds(0, HF), pl.ds(0, HD)], bd_v.at[1, pl.ds(0, HF), :]),
            (w2_hbm.at[pl.ds(HF, HF), pl.ds(0, HD)], sd_v.at[1]),
            (w2_hbm.at[pl.ds(0, HF), pl.ds(HD, HD)], sd_v.at[0]),
            (w2_hbm.at[pl.ds(HF, HF), pl.ds(HD, HD)], bd_v.at[4, pl.ds(0, HF), :]),
        )]
        for c in [cx0] + cst + cx + crest:
            c.start()

        def k_part(xi, a, b, first):
            pk = _phi(_dot(xi, wkv_v[:, a:b]))
            zs = jnp.sum(pk.reshape(pk.shape[0] // 8, 8, b - a), axis=0)
            if first:
                z_acc[:, a:b] = zs
            else:
                z_acc[:, a:b] += zs
            return pk.astype(BF)

        def kx_part(xi, pkb, a, b, first):
            kx = lax.dot_general(pkb, xi, (((0,), (0,)), ((), ())), preferred_element_type=F32)
            if first:
                kx_acc[a:b, :] = kx
            else:
                kx_acc[a:b, :] += kx

        with scope("p1_first"):
            prev = []
            for c in range(nchunks):
                with scope("w%d" % c):
                    if c == 0:
                        cx0.wait()
                    cst[c].wait()
                xi = x_v[0:r0, :]
                cur = (k_part(xi, pc[c], pc[c + 1], True), pc[c], pc[c + 1])
                for (pkb, a, b) in prev:
                    kx_part(xi, pkb, a, b, True)
                prev = [cur]
            for (pkb, a, b) in prev:
                kx_part(xi, pkb, a, b, True)

        def p1(i, carry):
            rr = pl.multiple_of(r0 + i * tm1, 16)
            pltpu.make_async_copy(x_hbm.at[pl.ds(rr, tm1)], x_v.at[pl.ds(rr, tm1)], sems.at[xbase + i]).wait()
            xi = x_v[pl.ds(rr, tm1), :]
            kx_part(xi, k_part(xi, 0, D, False), 0, D, False)
            return carry
        with scope("p1_rest"):
            lax.fori_loop(0, n1, p1, 0)

        with scope("wait_ffn"):
            for c in crest:
                c.wait()

        def w_combos(b11, b12, b21, b22):
            f = [t.astype(F32) for t in (b11, b12, b21, b22)]
            return {n: t.astype(BF) for n, t in enumerate(_b_combos(*f)) if n not in RAW}

        def pre_up(t, c):
            r = pl.ds(pl.multiple_of(t * 16, 16), 16)
            for c0 in range(0, WU, pcols):
                cs = slice(c0, c0 + pcols)
                for n, t_ in w_combos(bu_v[1, r, cs], su_v[0, r, cs], su_v[1, r, cs], bu_v[4, r, cs]).items():
                    bu_v[n, r, cs] = t_
            return c
        def pre_dn(t, c):
            for r1 in range(0, 64, 16):
                r = pl.ds(pl.multiple_of(t * 64 + r1, 16), 16)
                for n, t_ in w_combos(bd_v[1, r, :], sd_v[0, r, :], sd_v[1, r, :], bd_v[4, r, :]).items():
                    bd_v[n, r, :] = t_
            return c
        with scope("pre"):
            lax.fori_loop(0, HD // 16, pre_up, 0)
            lax.fori_loop(0, HF // 64, pre_dn, 0)

        with scope("mid"):
            ri = lax.broadcasted_iota(jnp.int32, (128, 128), 0) // DH
            ci = lax.broadcasted_iota(jnp.int32, (128, 128), 1) // DH
            same = ri == ci
            zr_v[...] = jnp.sum(z_acc[...], axis=0, keepdims=True)
            kvs = []
            for g in range(G):
                kvg = _dot(kx_acc[g * 128:(g + 1) * 128, :].astype(BF), wkv_v[:, D + g * 128:D + (g + 1) * 128])
                kvs.append(jnp.where(same, kvg, 0.0).astype(BF))
            for g in range(G // 2):
                mt = _dot(kvs[g], wo_v[g * 128:(g + 1) * 128, :])
                mb = _dot(kvs[g + 4], wo_v[(g + 4) * 128:(g + 5) * 128, :])
                for n, t_ in enumerate(_b_combos(mt[:, 0:HD], mt[:, HD:D], mb[:, 0:HD], mb[:, HD:D])):
                    bd_v[n, HF + g * 128:HF + (g + 1) * 128, :] = t_.astype(BF)

        oc = D // osplit
        def o_copy(rr, s):
            return pltpu.make_async_copy(o_v.at[pl.ds(rr, tm2), pl.ds(s * oc, oc)],
                                         o_hbm.at[pl.ds(rr, tm2), pl.ds(s * oc, oc)], osem)

        def p2(i, carry):
            rr = pl.multiple_of(i * tm2, tm2)
            xf = x_v[pl.ds(rr, tm2), :].astype(F32)
            gate = jax.nn.sigmoid(jnp.sum(xf * gw_v[...].astype(F32).reshape(1, D), axis=-1, keepdims=True))
            au = [t.astype(BF) for t in _a_combos(xf[0:hm, 0:HD], xf[0:hm, HD:D], xf[hm:tm2, 0:HD], xf[hm:tm2, HD:D])]
            gh = (gate[0:hm], gate[hm:tm2])

            def up_quads(c0, c1):
                return _c_combos(lambda n: _dot(au[n], bu_v[n, :, c0:c1]))

            pq = [[None] * G, [None] * G]
            for c0 in range(0, HD, fs):
                quads = up_quads(F + c0, F + c0 + fs)
                for half in range(2):
                    for side in range(2):
                        t_ = _phi(quads[2 * half + side])
                        for u in range(fs // 128):
                            pq[half][(side * HD + c0) // 128 + u] = t_[:, u * 128:(u + 1) * 128]

            def vpu_norm(half):
                lane = lax.broadcasted_iota(jnp.int32, (hm, 128), 1)
                zrow = zr_v[...]
                def swap(y, s):
                    return jnp.take_along_axis(y, lane ^ s, axis=1)
                cur = [pq[half][g] * zrow[:, g * 128:(g + 1) * 128] for g in range(G)]
                for s in (16, 8, 4):
                    m = (lane & s) == 0
                    n = len(cur) // 2
                    cur = [jnp.where(m, cur[t], cur[t + n]) + swap(jnp.where(m, cur[t + n], cur[t]), s)
                           for t in range(n)]
                y = cur[0]
                for s in (2, 1):
                    y = y + swap(y, s)
                r = gh[half] * pltpu.reciprocal(y + 1e-6, approx=True)
                return [pq[half][g] * jnp.take_along_axis(r, (lane & 96) + 4 * g, axis=1) for g in range(G)]

            def hchunk(c0, c1):
                c11, c12, c21, c22 = up_quads(c0, c1)
                def act(gt, up, g_):
                    return gt * pltpu.reciprocal(1.0 + jnp.exp(-gt), approx=True) * (up * (1.0 - g_))
                return act(c11, c12, gh[0]), act(c21, c22, gh[1])

            for j in range(HF // fs):
                c0, c1 = j * fs, (j + 1) * fs
                a11, a21 = hchunk(c0, c1)
                a12, a22 = hchunk(HF + c0, HF + c1)
                for n, t_ in enumerate(_a_combos(a11, a12, a21, a22)):
                    ad_v[n, :, c0:c1] = t_.astype(BF)
                if j + 1 == norm_at:
                    pt, pb = vpu_norm(0), vpu_norm(1)
                    for u in range(G // 2):
                        for n, t_ in enumerate(_a_combos(pt[u], pt[u + 4], pb[u], pb[u + 4])):
                            ad_v[n, :, HF + u * 128:HF + (u + 1) * 128] = t_.astype(BF)
            for s in range(osplit // 2):
                c0, c1 = s * oc, (s + 1) * oc
                c11, c12, c21, c22 = _c_combos(lambda n: _dot(ad_v[n], bd_v[n, :, c0:c1]))
                for (ct, cb, off) in ((c11, c21, 0), (c12, c22, HD)):
                    o_v[pl.ds(rr, tm2), off + c0:off + c1] = jnp.concatenate([ct, cb], axis=0).astype(BF)
                    o_copy(rr, (off + c0) // oc).start()
            return carry
        with scope("phase2"):
            lax.fori_loop(0, n2, p2, 0)
        with scope("tail"):
            pltpu.make_async_copy(o_v, o_hbm, osem).wait()

    def fn(A_x, A_wqkv, A_wo, B_x, B_w1, B_w3, B_w2, gate_w):
        x = A_x.reshape(S, D)
        anyspec = pl.BlockSpec(memory_space=pl.ANY)
        out = pl.pallas_call(
            kernel,
            in_specs=[anyspec] * 7,
            out_specs=anyspec,
            out_shape=jax.ShapeDtypeStruct((S, D), BF),
            scratch_shapes=[
                pltpu.VMEM((S, D), BF),
                pltpu.VMEM((D, 2 * D), BF),
                pltpu.VMEM((D, D), BF),
                pltpu.VMEM((7, HD, WU), BF),
                pltpu.VMEM((2, HD, WU), BF),
                pltpu.VMEM((7, KD, HD), BF),
                pltpu.VMEM((2, HF, HD), BF),
                pltpu.VMEM((D,), BF),
                pltpu.VMEM((S, D), BF),
                pltpu.VMEM((D, D), F32),
                pltpu.VMEM((8, D), F32),
                pltpu.VMEM((7, hm, KD), BF),
                pltpu.VMEM((1, D), F32),
                pltpu.SemaphoreType.DMA((nsem,)),
            ],
            compiler_params=pltpu.CompilerParams(vmem_limit_bytes=vmem_mb * 1024 * 1024),
        )(x, A_wqkv, A_wo, B_w1, B_w3, B_w2, gate_w)
        return out.reshape(1, S, D)
    return fn


_impl = make()


@jax.jit
def pallas_gated_mix__linear_attn_block__glu_gated_swiglu__prompt_kernel(
    A_x: jax.Array,
    A_wqkv: jax.Array,
    A_wo: jax.Array,
    B_x: jax.Array,
    B_w1: jax.Array,
    B_w3: jax.Array,
    B_w2: jax.Array,
    gate_w: jax.Array,
):
    return _impl(A_x, A_wqkv, A_wo, B_x, B_w1, B_w3, B_w2, gate_w)
```

```python
import contextlib
import jax
import jax.numpy as jnp
import numpy as np
from jax import lax
from jax.experimental import pallas as pl
from jax.experimental.pallas import tpu as pltpu

BF = jnp.bfloat16
F32 = jnp.float32


def _phi(t):
    return jnp.where(t > 0, t + 1.0, jnp.exp(t)) + 1e-6


def _dot(a, b):
    return jnp.dot(a, b, preferred_element_type=F32)


def _a_combos(a11, a12, a21, a22):
    return [a11 + a22, a21 + a22, a11, a22, a11 + a12, a21 - a11, a12 - a22]


def _b_combos(b11, b12, b21, b22):
    return [b11 + b22, b11, b12 - b22, b21 - b11, b22, b11 + b12, b21 + b22]


def _c_combos(prod, order=(0, 3, 4, 6, 1, 2, 5)):
    m = {n: prod(n) for n in order}
    return (m[0] + m[3] - m[4] + m[6], m[2] + m[4], m[1] + m[3], m[0] - m[1] + m[2] + m[5])


def make(r0=128, tm1=384, tm2=256, fs=256, plan=(256, 512, 768, 1024),
         vmem_mb=120, scopes=False, norm_at=1, osplit=4, pcols=512, npc=1, kshare=0.25, cut=0.85, grp=1, cr=352):
    S, D, F, H = 2048, 1024, 3584, 32
    DH = D // H
    G = D // 128
    HD, HF = D // 2, F // 2
    WU = F + HD
    KD = HF + HD
    n1 = (S - r0) // tm1
    assert r0 + n1 * tm1 == S
    n2 = S // tm2
    hm = tm2 // 2
    scope = (lambda n: jax.named_scope(n)) if scopes else (lambda n: contextlib.nullcontext())
    pc = [0] + list(plan)
    nchunks = len(plan)
    NC = n1 - 1
    CW = WU // NC
    CR = cr
    CM = HF - NC * CR
    assert CW * NC == WU and CM >= 0 and CW % 128 == 0 and CR % 16 == 0
    nsem = 1 + nchunks + n1 + NC + 2
    RAW = (1, 4)

    def kernel(x_hbm, wqkv_hbm, wo_hbm, w1_hbm, w3_hbm, w2_hbm, gw_hbm, o_hbm,
               x_v, wkv_v, wo_v, bu_v, su_v, bd_v, sd_v, gw_v, o_v, kx_acc, z_acc, ad_v, zr_v, zero_v,
               sems):
        ctr = [0]
        def mk(src, dst):
            c = pltpu.make_async_copy(src, dst, sems.at[ctr[0]])
            ctr[0] += 1
            return c
        cx0 = mk(x_hbm.at[pl.ds(0, r0)], x_v.at[pl.ds(0, r0)])
        cst = [mk(wqkv_hbm.at[:, pl.ds(D + pc[c], pc[c + 1] - pc[c])], wkv_v.at[:, pl.ds(pc[c], pc[c + 1] - pc[c])])
               for c in range(nchunks)]
        xbase = ctr[0]
        wbase = xbase + n1
        rsem = sems.at[wbase + NC]
        osem = sems.at[wbase + NC + 1]

        def x_copy(i):
            rr = r0 + i * tm1
            if not isinstance(i, int):
                rr = pl.multiple_of(rr, 16)
            return pltpu.make_async_copy(x_hbm.at[pl.ds(rr, tm1)], x_v.at[pl.ds(rr, tm1)], sems.at[xbase + i])

        NP = 2
        PW = CW // NP
        assert F % PW == 0
        def w_copies(c, real):
            sem = sems.at[wbase + c]
            out = []
            for p in range(NP):
                for (dst, slot, left, rows0) in ((bu_v, 1, True, 0), (su_v, 1, True, HD), (su_v, 0, False, 0), (bu_v, 4, False, HD)):
                    d = dst.at[c, slot, :, pl.ds(p * PW, PW)]
                    if real:
                        col = c * CW + p * PW
                        if col < F:
                            src = (w1_hbm if left else w3_hbm).at[pl.ds(rows0, HD), pl.ds(col, PW)]
                        else:
                            src = wqkv_hbm.at[pl.ds(rows0, HD), pl.ds(col - F + (0 if left else HD), PW)]
                    else:
                        src = w1_hbm.at[pl.ds(rows0, HD), pl.ds(0, PW)]
                    out.append(pltpu.make_async_copy(src, d, sem))
            rr = c * CR if real else pl.multiple_of(c * CR, 16)
            for (dst, slot, r0_, c0_) in ((bd_v, 1, 0, 0), (sd_v, 1, HF, 0), (sd_v, 0, 0, HD), (bd_v, 4, HF, HD)):
                src = w2_hbm.at[pl.ds(r0_ + (c * CR if real else 0), CR), pl.ds(c0_, HD)]
                out.append(pltpu.make_async_copy(src, dst.at[slot, pl.ds(rr, CR), :], sem))
            return out

        crest = [pltpu.make_async_copy(a_, b_, rsem) for (a_, b_) in (
            (gw_hbm, gw_v),
            (wqkv_hbm.at[:, pl.ds(2 * D, D)], wkv_v.at[:, pl.ds(D, D)]),
            (wo_hbm, wo_v))]
        if CM:
            crest = [pltpu.make_async_copy(w2_hbm.at[pl.ds(r0_ + NC * CR, CM), pl.ds(c0_, HD)],
                                           dst.at[slot, pl.ds(NC * CR, CM), :], rsem)
                     for (dst, slot, r0_, c0_) in ((bd_v, 1, 0, 0), (sd_v, 1, HF, 0), (sd_v, 0, 0, HD), (bd_v, 4, HF, HD))] + crest
        order = [cx0] + cst + [x_copy(0)]
        for c in range(NC):
            order += [x_copy(c + 1)] + w_copies(c, True)
        for c in order + crest:
            c.start()

        def k_part(xi, a, b, first):
            pk = _phi(_dot(xi, wkv_v[:, a:b]))
            zs = jnp.sum(pk.reshape(pk.shape[0] // 8, 8, b - a), axis=0)
            if first:
                z_acc[:, a:b] = zs
            else:
                z_acc[:, a:b] += zs
            return pk.astype(BF), pk

        def kx_part(xi, pkb, a, b, first):
            kx = lax.dot_general(pkb, xi, (((0,), (0,)), ((), ())), preferred_element_type=F32)
            if first:
                kx_acc[a:b, :] = kx
            else:
                kx_acc[a:b, :] += kx
            return kx

        zero_v[...] = jnp.zeros((16, 128), jnp.int32)
        with scope("p1_first"):
            prev = []
            for c in range(nchunks):
                with scope("w%d" % c):
                    if c == 0:
                        cx0.wait()
                    cst[c].wait()
                xi = x_v[0:r0, :]
                cur = (k_part(xi, pc[c], pc[c + 1], True)[0], pc[c], pc[c + 1])
                for (pkb, a, b) in prev:
                    kx_part(xi, pkb, a, b, True)
                prev = [cur]
            for (pkb, a, b) in prev:
                kx_part(xi, pkb, a, b, True)

        def w_combos(b11, b12, b21, b22, tie=None):
            f = [t.astype(F32) for t in (b11, b12, b21, b22)]
            if tie is not None:
                f[0] = f[0] + tie
                f[3] = f[3] + tie
            return {n: t.astype(BF) for n, t in enumerate(_b_combos(*f)) if n not in RAW}

        def pre_up(cc, r_lo, r_hi):
            for r1 in range(r_lo, r_hi, 16):
                for c0 in range(0, CW, pcols):
                    r, cs = slice(r1, r1 + 16), slice(c0, c0 + pcols)
                    for n, t_ in w_combos(bu_v[cc, 1, r, cs], su_v[cc, 0, r, cs], su_v[cc, 1, r, cs], bu_v[cc, 4, r, cs], tie).items():
                        bu_v[cc, n, r, cs] = t_
        def pre_dn(ro, so, lo, hi):
            for r1 in range(lo, hi, 16):
                r = pl.ds(ro + r1, 16)
                q = pl.ds(so + r1, 16)
                for n, t_ in w_combos(bd_v[1, r, :], sd_v[0, q, :], sd_v[1, q, :], bd_v[4, r, :]).items():
                    bd_v[n, r, :] = t_

        def p1(i, carry):
            rr = pl.multiple_of(r0 + i * tm1, 16)
            x_copy(i).wait()
            @pl.when(i > 0)
            def _():
                for c in w_copies(i - 1, False):
                    c.wait()
            cc = jnp.where(i == 0, NC, i - 1)
            ro = pl.multiple_of(jnp.where(i == 0, KD, (i - 1) * CR), 16)
            so = pl.multiple_of(cc * CR, 16)
            xi = x_v[pl.ds(rr, tm1), :]
            todo = [('u', r1, c0) for r1 in range(0, HD, 16) for c0 in range(0, CW, 128)]
            todo += [('d', r1, c0) for r1 in range(0, CR, 16) for c0 in range(0, HD, 128)]
            zero = zero_v[...]
            def do(kind, r1, c0, tie):
                cs = slice(c0, c0 + 128)
                if kind == 'u':
                    r = slice(r1, r1 + 16)
                    for n, t_ in w_combos(bu_v[cc, 1, r, cs], su_v[cc, 0, r, cs], su_v[cc, 1, r, cs], bu_v[cc, 4, r, cs], tie).items():
                        bu_v[cc, n, r, cs] = t_
                else:
                    r, q = pl.ds(ro + r1, 16), pl.ds(so + r1, 16)
                    for n, t_ in w_combos(bd_v[1, r, cs], sd_v[0, q, cs], sd_v[1, q, cs], bd_v[4, r, cs], tie).items():
                        bd_v[n, r, cs] = t_
            state = [0, 0.0]
            def paced(val, share):
                tiles = [(r1, c0) for c0 in range(0, val.shape[1], 128) for r1 in range(0, val.shape[0], 16)]
                for k, (r1, c0) in enumerate(tiles):
                    goal = int(round((state[1] + share * min(1.0, (k + 1) / (len(tiles) * cut))) * len(todo)))
                    if goal >= state[0] + grp or (goal == len(todo) and goal > state[0]):
                        v = val[r1:r1 + 16, c0:c0 + 128]
                        tie = lax.bitcast_convert_type(lax.bitcast_convert_type(v, jnp.int32) & zero, F32)
                        while state[0] < goal:
                            do(*todo[state[0]], tie)
                            state[0] += 1
                state[1] += share
            NPC = npc
            w = D // NPC
            shk, shx = kshare / NPC, (1.0 - kshare) / NPC
            pend = None
            for c in range(NPC):
                pkb, pkf = k_part(xi, c * w, (c + 1) * w, False)
                paced(pkf, shk)
                if pend is not None:
                    paced(kx_part(xi, *pend, False), shx)
                pend = (pkb, c * w, (c + 1) * w)
            paced(kx_part(xi, *pend, False), shx)
            assert state[0] == len(todo)
            return carry
        with scope("p1_rest"):
            lax.fori_loop(0, n1, p1, 0)

        with scope("wait_ffn"):
            for c in crest:
                c.wait()

        with scope("mid"):
            ri = lax.broadcasted_iota(jnp.int32, (128, 128), 0) // DH
            ci = lax.broadcasted_iota(jnp.int32, (128, 128), 1) // DH
            same = ri == ci
            zr_v[...] = jnp.sum(z_acc[...], axis=0, keepdims=True)
            kvs, kvf = [], []
            for g in range(G):
                kvg = _dot(kx_acc[g * 128:(g + 1) * 128, :].astype(BF), wkv_v[:, D + g * 128:D + (g + 1) * 128])
                kvs.append(jnp.where(same, kvg, 0.0).astype(BF))
                kvf.append(kvg)
            todo2 = [(r1, c0) for r1 in range(NC * CR, HF, 16) for c0 in range(0, HD, 128)]
            st2 = [0]
            zero2 = zero_v[...]
            def paced2(val, frac):
                goal = int(round(frac * len(todo2)))
                if goal > st2[0]:
                    tie = lax.bitcast_convert_type(lax.bitcast_convert_type(val, jnp.int32) & zero2, F32)
                    while st2[0] < goal:
                        r1, c0 = todo2[st2[0]]
                        r, cs = slice(r1, r1 + 16), slice(c0, c0 + 128)
                        for n, t_ in w_combos(bd_v[1, r, cs], sd_v[0, r, cs], sd_v[1, r, cs], bd_v[4, r, cs], tie).items():
                            bd_v[n, r, cs] = t_
                        st2[0] += 1
            for g in range(G):
                for u in range(8):
                    paced2(kvf[g][u * 16:(u + 1) * 16, :], (g * 8 + u + 1) / 64.0)
            for g in range(G // 2):
                mt = _dot(kvs[g], wo_v[g * 128:(g + 1) * 128, :])
                mb = _dot(kvs[g + 4], wo_v[(g + 4) * 128:(g + 5) * 128, :])
                for n, t_ in enumerate(_b_combos(mt[:, 0:HD], mt[:, HD:D], mb[:, 0:HD], mb[:, HD:D])):
                    bd_v[n, HF + g * 128:HF + (g + 1) * 128, :] = t_.astype(BF)

        oc = D // osplit
        def o_copy(rr, s):
            return pltpu.make_async_copy(o_v.at[pl.ds(rr, tm2), pl.ds(s * oc, oc)],
                                         o_hbm.at[pl.ds(rr, tm2), pl.ds(s * oc, oc)], osem)

        def p2(i, carry):
            rr = pl.multiple_of(i * tm2, tm2)
            xf = x_v[pl.ds(rr, tm2), :].astype(F32)
            gate = jax.nn.sigmoid(jnp.sum(xf * gw_v[...].astype(F32).reshape(1, D), axis=-1, keepdims=True))
            au = [t.astype(BF) for t in _a_combos(xf[0:hm, 0:HD], xf[0:hm, HD:D], xf[hm:tm2, 0:HD], xf[hm:tm2, HD:D])]
            gh = (gate[0:hm], gate[hm:tm2])

            def up_quads(c0, c1):
                return _c_combos(lambda n: _dot(au[n], bu_v[c0 // CW, n, :, c0 % CW:c0 % CW + (c1 - c0)]))

            pq = [[None] * G, [None] * G]
            for c0 in range(0, HD, fs):
                quads = up_quads(F + c0, F + c0 + fs)
                for half in range(2):
                    for side in range(2):
                        t_ = _phi(quads[2 * half + side])
                        for u in range(fs // 128):
                            pq[half][(side * HD + c0) // 128 + u] = t_[:, u * 128:(u + 1) * 128]

            def vpu_norm(half):
                lane = lax.broadcasted_iota(jnp.int32, (hm, 128), 1)
                zrow = zr_v[...]
                def swap(y, s):
                    return jnp.take_along_axis(y, lane ^ s, axis=1)
                cur = [pq[half][g] * zrow[:, g * 128:(g + 1) * 128] for g in range(G)]
                for s in (16, 8, 4):
                    m = (lane & s) == 0
                    n = len(cur) // 2
                    cur = [jnp.where(m, cur[t], cur[t + n]) + swap(jnp.where(m, cur[t + n], cur[t]), s)
                           for t in range(n)]
                y = cur[0]
                for s in (2, 1):
                    y = y + swap(y, s)
                r = gh[half] * pltpu.reciprocal(y + 1e-6, approx=True)
                return [pq[half][g] * jnp.take_along_axis(r, (lane & 96) + 4 * g, axis=1) for g in range(G)]

            def hchunk(c0, c1):
                c11, c12, c21, c22 = up_quads(c0, c1)
                def act(gt, up, g_):
                    return gt * pltpu.reciprocal(1.0 + jnp.exp(-gt), approx=True) * (up * (1.0 - g_))
                return act(c11, c12, gh[0]), act(c21, c22, gh[1])

            for j in range(HF // fs):
                c0, c1 = j * fs, (j + 1) * fs
                a11, a21 = hchunk(c0, c1)
                a12, a22 = hchunk(HF + c0, HF + c1)
                for n, t_ in enumerate(_a_combos(a11, a12, a21, a22)):
                    ad_v[n, :, c0:c1] = t_.astype(BF)
                if j + 1 == norm_at:
                    pt, pb = vpu_norm(0), vpu_norm(1)
                    for u in range(G // 2):
                        for n, t_ in enumerate(_a_combos(pt[u], pt[u + 4], pb[u], pb[u + 4])):
                            ad_v[n, :, HF + u * 128:HF + (u + 1) * 128] = t_.astype(BF)
            for s in range(osplit // 2):
                c0, c1 = s * oc, (s + 1) * oc
                c11, c12, c21, c22 = _c_combos(lambda n: _dot(ad_v[n], bd_v[n, 0:KD, c0:c1]))
                for (ct, cb, off) in ((c11, c21, 0), (c12, c22, HD)):
                    o_v[pl.ds(rr, tm2), off + c0:off + c1] = jnp.concatenate([ct, cb], axis=0).astype(BF)
                    o_copy(rr, (off + c0) // oc).start()
            return carry
        with scope("phase2"):
            lax.fori_loop(0, n2, p2, 0)
        with scope("tail"):
            pltpu.make_async_copy(o_v, o_hbm, osem).wait()

    def fn(A_x, A_wqkv, A_wo, B_x, B_w1, B_w3, B_w2, gate_w):
        x = A_x.reshape(S, D)
        anyspec = pl.BlockSpec(memory_space=pl.ANY)
        out = pl.pallas_call(
            kernel,
            in_specs=[anyspec] * 7,
            out_specs=anyspec,
            out_shape=jax.ShapeDtypeStruct((S, D), BF),
            scratch_shapes=[
                pltpu.VMEM((S, D), BF),
                pltpu.VMEM((D, 2 * D), BF),
                pltpu.VMEM((D, D), BF),
                pltpu.VMEM((NC + 1, 7, HD, CW), BF),
                pltpu.VMEM((NC + 1, 2, HD, CW), BF),
                pltpu.VMEM((7, KD + CR, HD), BF),
                pltpu.VMEM((2, HF + CR, HD), BF),
                pltpu.VMEM((D,), BF),
                pltpu.VMEM((S, D), BF),
                pltpu.VMEM((D, D), F32),
                pltpu.VMEM((8, D), F32),
                pltpu.VMEM((7, hm, KD), BF),
                pltpu.VMEM((1, D), F32),
                pltpu.VMEM((16, 128), jnp.int32),
                pltpu.SemaphoreType.DMA((nsem,)),
            ],
            compiler_params=pltpu.CompilerParams(vmem_limit_bytes=vmem_mb * 1024 * 1024),
        )(x, A_wqkv, A_wo, B_w1, B_w3, B_w2, gate_w)
        return out.reshape(1, S, D)
    return fn


_impl = make(cr=352)


@jax.jit
def pallas_gated_mix__linear_attn_block__glu_gated_swiglu__prompt_kernel(
    A_x: jax.Array,
    A_wqkv: jax.Array,
    A_wo: jax.Array,
    B_x: jax.Array,
    B_w1: jax.Array,
    B_w3: jax.Array,
    B_w2: jax.Array,
    gate_w: jax.Array,
):
    return _impl(A_x, A_wqkv, A_wo, B_x, B_w1, B_w3, B_w2, gate_w)
```

```python
import contextlib
import jax
import jax.numpy as jnp
import numpy as np
from jax import lax
from jax.experimental import pallas as pl
from jax.experimental.pallas import tpu as pltpu

BF = jnp.bfloat16
F32 = jnp.float32


def _phi(t):
    return jnp.where(t > 0, t + 1.0, jnp.exp(t)) + 1e-6


def _dot(a, b):
    return jnp.dot(a, b, preferred_element_type=F32)


def _a_combos(a11, a12, a21, a22):
    return [a11 + a22, a21 + a22, a11, a22, a11 + a12, a21 - a11, a12 - a22]


def _b_combos(b11, b12, b21, b22):
    return [b11 + b22, b11, b12 - b22, b21 - b11, b22, b11 + b12, b21 + b22]


def _c_combos(prod, order=(0, 3, 4, 6, 1, 2, 5)):
    m = {n: prod(n) for n in order}
    return (m[0] + m[3] - m[4] + m[6], m[2] + m[4], m[1] + m[3], m[0] - m[1] + m[2] + m[5])


def make(r0=128, tm1=384, tm2=256, fs=256, plan=(256, 512, 768, 1024),
         vmem_mb=120, scopes=False, norm_at=1, osplit=4, pcols=512, npc=1, kshare=0.15, cut=0.85, grp=1, cr=320, kc=256, k0cut=6, mcut=0.85, mfa=0.5):
    S, D, F, H = 2048, 1024, 3584, 32
    DH = D // H
    G = D // 128
    HD, HF = D // 2, F // 2
    WU = F + HD
    KD = HF + HD
    n1 = (S - r0) // tm1
    assert r0 + n1 * tm1 == S
    n2 = S // tm2
    hm = tm2 // 2
    scope = (lambda n: jax.named_scope(n)) if scopes else (lambda n: contextlib.nullcontext())
    pc = [0] + list(plan)
    nchunks = len(plan)
    kcols = ((0, 256), (512, 768), (256, 512), (768, 1024))
    NC = n1 - 1
    CW = WU // NC
    CR = cr
    CM = HF - NC * CR
    assert CW * NC == WU and CM >= 0 and CW % 128 == 0 and CR % 16 == 0
    nsem = 1 + nchunks + n1 + NC + 3
    RAW = (1, 4)

    def kernel(x_hbm, wqkv_hbm, wo_hbm, w1_hbm, w3_hbm, w2_hbm, gw_hbm, o_hbm,
               x_v, wkv_v, wo_v, bu_v, su_v, bd_v, sd_v, gw_v, o_v, kx_acc, z_acc, ad_v, zr_v, zero_v, bk_v,
               sems):
        ctr = [0]
        def mk(src, dst):
            c = pltpu.make_async_copy(src, dst, sems.at[ctr[0]])
            ctr[0] += 1
            return c
        cx0 = mk(x_hbm.at[pl.ds(0, r0)], x_v.at[pl.ds(0, r0)])
        cst = [mk(wqkv_hbm.at[:, pl.ds(D + a_, b_ - a_)], wkv_v.at[:, pl.ds(a_, b_ - a_)]) for (a_, b_) in kcols]
        xbase = ctr[0]
        wbase = xbase + n1
        rsem = sems.at[wbase + NC]
        osem = sems.at[wbase + NC + 1]

        def x_copy(i):
            rr = r0 + i * tm1
            if not isinstance(i, int):
                rr = pl.multiple_of(rr, 16)
            return pltpu.make_async_copy(x_hbm.at[pl.ds(rr, tm1)], x_v.at[pl.ds(rr, tm1)], sems.at[xbase + i])

        NP = 2
        PW = CW // NP
        assert F % PW == 0
        def w_copies(c, real):
            sem = sems.at[wbase + c]
            out = []
            for p in range(NP):
                for (dst, slot, left, rows0) in ((bu_v, 1, True, 0), (su_v, 1, True, HD), (su_v, 0, False, 0), (bu_v, 4, False, HD)):
                    d = dst.at[c, slot, :, pl.ds(p * PW, PW)]
                    if real:
                        col = c * CW + p * PW
                        if col < F:
                            src = (w1_hbm if left else w3_hbm).at[pl.ds(rows0, HD), pl.ds(col, PW)]
                        else:
                            src = wqkv_hbm.at[pl.ds(rows0, HD), pl.ds(col - F + (0 if left else HD), PW)]
                    else:
                        src = w1_hbm.at[pl.ds(rows0, HD), pl.ds(0, PW)]
                    out.append(pltpu.make_async_copy(src, d, sem))
            rr = c * CR if real else pl.multiple_of(c * CR, 16)
            for (dst, slot, r0_, c0_) in ((bd_v, 1, 0, 0), (sd_v, 1, HF, 0), (sd_v, 0, 0, HD), (bd_v, 4, HF, HD)):
                src = w2_hbm.at[pl.ds(r0_ + (c * CR if real else 0), CR), pl.ds(c0_, HD)]
                out.append(pltpu.make_async_copy(src, dst.at[slot, pl.ds(rr, CR), :], sem))
            return out

        crest = [pltpu.make_async_copy(a_, b_, rsem) for (a_, b_) in (
            (gw_hbm, gw_v),
            (wqkv_hbm.at[:, pl.ds(2 * D, D)], wkv_v.at[:, pl.ds(D, D)]))]
        mk_wo = pltpu.make_async_copy(wo_hbm, wo_v, rsem)
        CMA = int(CM * mfa) // 16 * 16
        def cm_copies(lo, n, sem):
            return [pltpu.make_async_copy(w2_hbm.at[pl.ds(r0_ + lo, n), pl.ds(c0_, HD)], dst.at[slot, pl.ds(lo, n), :], sem)
                    for (dst, slot, r0_, c0_) in ((bd_v, 1, 0, 0), (sd_v, 1, HF, 0), (sd_v, 0, 0, HD), (bd_v, 4, HF, HD))]
        crest = crest + [mk_wo] + cm_copies(NC * CR, CMA, rsem)
        clast = cm_copies(NC * CR + CMA, CM - CMA, sems.at[wbase + NC + 2])
        order = [cx0] + cst + [x_copy(0)]
        for c in range(NC):
            order += [x_copy(c + 1)] + w_copies(c, True)
        for c in order + crest + clast:
            c.start()

        def w_combos(b11, b12, b21, b22, tie=None):
            f = [t.astype(F32) for t in (b11, b12, b21, b22)]
            if tie is not None:
                f[0] = f[0] + tie
                f[3] = f[3] + tie
            return {n: t.astype(BF) for n, t in enumerate(_b_combos(*f)) if n not in RAW}

        def k_part(xi, a, b, first):
            pk = _phi(_dot(xi, wkv_v[:, a:b]))
            zs = jnp.sum(pk.reshape(pk.shape[0] // 8, 8, b - a), axis=0)
            if first:
                z_acc[:, a:b] = zs
            else:
                z_acc[:, a:b] += zs
            return pk.astype(BF), pk

        def kx_part(xi, pkb, a, b, first):
            kx = lax.dot_general(pkb, xi, (((0,), (0,)), ((), ())), preferred_element_type=F32)
            if first:
                kx_acc[a:b, :] = kx
            else:
                kx_acc[a:b, :] += kx
            return kx

        zero_v[...] = jnp.zeros((16, 128), jnp.int32)
        with scope("p1_first"):
            zero0 = zero_v[...]
            def wk_sums(lo, hi, val):
                todo0 = [(r1, c0) for c0 in range(lo, hi, 128) for r1 in range(0, HD, 16)]
                tiles0 = [(r1, c0) for c0 in range(0, val.shape[1], 128) for r1 in range(0, val.shape[0], 16)]
                tiles0 = tiles0[:max(1, len(tiles0) * k0cut // 8)]
                per = -(-len(todo0) // len(tiles0))
                for (r1, c0) in tiles0:
                    part, todo0 = todo0[:per], todo0[per:]
                    if part:
                        tie = lax.bitcast_convert_type(lax.bitcast_convert_type(val[r1:r1 + 16, c0:c0 + 128], jnp.int32) & zero0, F32)
                    for (q1, d0) in part:
                        r, r2, cs, cs2 = slice(q1, q1 + 16), slice(HD + q1, HD + q1 + 16), slice(d0, d0 + 128), slice(HD + d0, HD + d0 + 128)
                        for n, t_ in w_combos(wkv_v[r, cs], wkv_v[r, cs2], wkv_v[r2, cs], wkv_v[r2, cs2], tie).items():
                            bk_v[n, r, cs] = t_
                assert not todo0
            prev = None
            for c in range(nchunks):
                with scope("w%d" % c):
                    if c == 0:
                        cx0.wait()
                    cst[c].wait()
                a, b = kcols[c]
                xi = x_v[0:r0, :]
                pkb, pkf = k_part(xi, a, b, True)
                if c == 1:
                    wk_sums(a - HD, b - HD, pkf)
                if prev is not None:
                    kx_part(xi, *prev, True)
                prev = (pkb, a, b)
            kx = kx_part(xi, *prev, True)
            wk_sums(prev[1] - HD, prev[2] - HD, kx)

        def pre_up(cc, r_lo, r_hi):
            for r1 in range(r_lo, r_hi, 16):
                for c0 in range(0, CW, pcols):
                    r, cs = slice(r1, r1 + 16), slice(c0, c0 + pcols)
                    for n, t_ in w_combos(bu_v[cc, 1, r, cs], su_v[cc, 0, r, cs], su_v[cc, 1, r, cs], bu_v[cc, 4, r, cs], tie).items():
                        bu_v[cc, n, r, cs] = t_
        def pre_dn(ro, so, lo, hi):
            for r1 in range(lo, hi, 16):
                r = pl.ds(ro + r1, 16)
                q = pl.ds(so + r1, 16)
                for n, t_ in w_combos(bd_v[1, r, :], sd_v[0, q, :], sd_v[1, q, :], bd_v[4, r, :]).items():
                    bd_v[n, r, :] = t_

        def p1(i, carry):
            rr = pl.multiple_of(r0 + i * tm1, 16)
            x_copy(i).wait()
            @pl.when(i > 0)
            def _():
                for c in w_copies(i - 1, False):
                    c.wait()
            cc = jnp.where(i == 0, NC, i - 1)
            ro = pl.multiple_of(jnp.where(i == 0, KD, (i - 1) * CR), 16)
            so = pl.multiple_of(jnp.where(i == 0, HF, (i - 1) * CR), 16)
            xi = x_v[pl.ds(rr, tm1), :]
            todo = [('u', r1, c0) for r1 in range(0, HD, 16) for c0 in range(0, CW, 128)]
            todo += [('d', r1, c0) for r1 in range(0, CR, 16) for c0 in range(0, HD, 128)]
            zero = zero_v[...]
            def do(kind, r1, c0, tie):
                cs = slice(c0, c0 + 128)
                if kind == 'u':
                    r = slice(r1, r1 + 16)
                    for n, t_ in w_combos(bu_v[cc, 1, r, cs], su_v[cc, 0, r, cs], su_v[cc, 1, r, cs], bu_v[cc, 4, r, cs], tie).items():
                        bu_v[cc, n, r, cs] = t_
                else:
                    r, q = pl.ds(ro + r1, 16), pl.ds(so + r1, 16)
                    for n, t_ in w_combos(bd_v[1, r, cs], sd_v[0, q, cs], sd_v[1, q, cs], bd_v[4, r, cs], tie).items():
                        bd_v[n, r, cs] = t_
            state = [0, 0.0]
            def paced(val, share):
                tiles = [(r1, c0) for c0 in range(0, val.shape[1], 128) for r1 in range(0, val.shape[0], 16)]
                for k, (r1, c0) in enumerate(tiles):
                    goal = int(round((state[1] + share * min(1.0, (k + 1) / (len(tiles) * cut))) * len(todo)))
                    if goal >= state[0] + grp or (goal == len(todo) and goal > state[0]):
                        v = val[r1:r1 + 16, c0:c0 + 128]
                        tie = lax.bitcast_convert_type(lax.bitcast_convert_type(v, jnp.int32) & zero, F32)
                        while state[0] < goal:
                            do(*todo[state[0]], tie)
                            state[0] += 1
                state[1] += share
            NPC = npc
            w = D // NPC
            shk, shx = kshare / NPC, (1.0 - kshare) / NPC
            hr = tm1 // 2
            xf = xi.astype(F32)
            xa = [t.astype(BF) for t in _a_combos(xf[0:hr, 0:HD], xf[0:hr, HD:D], xf[hr:tm1, 0:HD], xf[hr:tm1, HD:D])]
            def bk(n, c0, c1):
                if n == 1:
                    return wkv_v[0:HD, c0:c1]
                if n == 4:
                    return wkv_v[HD:D, HD + c0:HD + c1]
                return bk_v[n, :, c0:c1]
            pkq = [[], [], [], []]
            for c0 in range(0, HD, kc):
                quads = _c_combos(lambda n: _dot(xa[n], bk(n, c0, c0 + kc)))
                for q in range(4):
                    pkq[q].append(_phi(quads[q]))
                for side in range(2):
                    zs = pkq[side][-1] + pkq[2 + side][-1]
                    z_acc[:, side * HD + c0:side * HD + c0 + kc] += jnp.sum(zs.reshape(hr // 8, 8, kc), axis=0)
                paced(pkq[3][-1], kshare * kc / HD)
            pq_ = [p[0] if len(p) == 1 else jnp.concatenate(p, axis=1) for p in pkq]
            pkb = jnp.concatenate([jnp.concatenate([pq_[0], pq_[1]], axis=1), jnp.concatenate([pq_[2], pq_[3]], axis=1)], axis=0).astype(BF)
            paced(kx_part(xi, pkb, 0, D, False), 1.0 - kshare)
            assert state[0] == len(todo)
            return carry
        with scope("p1_rest"):
            lax.fori_loop(0, n1, p1, 0)

        with scope("wait_ffn"):
            for c in crest:
                c.wait()

        with scope("mid"):
            ri = lax.broadcasted_iota(jnp.int32, (128, 128), 0) // DH
            ci = lax.broadcasted_iota(jnp.int32, (128, 128), 1) // DH
            same = ri == ci
            zr_v[...] = jnp.sum(z_acc[...], axis=0, keepdims=True)
            kvs, kvf = [], []
            for g in range(G):
                kvg = _dot(kx_acc[g * 128:(g + 1) * 128, :].astype(BF), wkv_v[:, D + g * 128:D + (g + 1) * 128])
                kvs.append(jnp.where(same, kvg, 0.0).astype(BF))
                kvf.append(kvg)
            todo2 = [(r1, c0) for r1 in range(NC * CR, HF, 16) for c0 in range(0, HD, 128)]
            st2 = [0]
            zero2 = zero_v[...]
            def paced2(val, frac):
                goal = int(round(frac * len(todo2)))
                if goal > st2[0]:
                    tie = lax.bitcast_convert_type(lax.bitcast_convert_type(val, jnp.int32) & zero2, F32)
                    while st2[0] < goal:
                        r1, c0 = todo2[st2[0]]
                        r, cs = slice(r1, r1 + 16), slice(c0, c0 + 128)
                        for n, t_ in w_combos(bd_v[1, r, cs], sd_v[0, r, cs], sd_v[1, r, cs], bd_v[4, r, cs], tie).items():
                            bd_v[n, r, cs] = t_
                        st2[0] += 1
            fa = CMA / CM
            for g in range(G):
                for u in range(8):
                    paced2(kvf[g][u * 16:(u + 1) * 16, :], fa * (g * 8 + u + 1) / 64.0)
            for c in clast:
                c.wait()
            for g in range(G // 2):
                mt = _dot(kvs[g], wo_v[g * 128:(g + 1) * 128, :])
                mb = _dot(kvs[g + 4], wo_v[(g + 4) * 128:(g + 5) * 128, :])
                for n, t_ in enumerate(_b_combos(mt[:, 0:HD], mt[:, HD:D], mb[:, 0:HD], mb[:, HD:D])):
                    bd_v[n, HF + g * 128:HF + (g + 1) * 128, :] = t_.astype(BF)
                for w_, mm in enumerate((mt, mb)):
                    for u in range(8):
                        for v_ in range(0, 128, 64):
                            k_ = ((g * 2 + w_) * 8 + u) * 2 + v_ // 64 + 1
                            paced2(mm[v_:v_ + 16, u * 128:(u + 1) * 128], min(1.0, fa + (1 - fa) * k_ / (128.0 * mcut)))
            assert st2[0] == len(todo2)

        oc = D // osplit
        def o_copy(rr, s):
            return pltpu.make_async_copy(o_v.at[pl.ds(rr, tm2), pl.ds(s * oc, oc)],
                                         o_hbm.at[pl.ds(rr, tm2), pl.ds(s * oc, oc)], osem)

        def p2(i, carry):
            rr = pl.multiple_of(i * tm2, tm2)
            xf = x_v[pl.ds(rr, tm2), :].astype(F32)
            gate = jax.nn.sigmoid(jnp.sum(xf * gw_v[...].astype(F32).reshape(1, D), axis=-1, keepdims=True))
            au = [t.astype(BF) for t in _a_combos(xf[0:hm, 0:HD], xf[0:hm, HD:D], xf[hm:tm2, 0:HD], xf[hm:tm2, HD:D])]
            gh = (gate[0:hm], gate[hm:tm2])

            def up_quads(c0, c1):
                return _c_combos(lambda n: _dot(au[n], bu_v[c0 // CW, n, :, c0 % CW:c0 % CW + (c1 - c0)]))

            pq = [[None] * G, [None] * G]
            for c0 in range(0, HD, fs):
                quads = up_quads(F + c0, F + c0 + fs)
                for half in range(2):
                    for side in range(2):
                        t_ = _phi(quads[2 * half + side])
                        for u in range(fs // 128):
                            pq[half][(side * HD + c0) // 128 + u] = t_[:, u * 128:(u + 1) * 128]

            def vpu_norm(half):
                lane = lax.broadcasted_iota(jnp.int32, (hm, 128), 1)
                zrow = zr_v[...]
                def swap(y, s):
                    return jnp.take_along_axis(y, lane ^ s, axis=1)
                cur = [pq[half][g] * zrow[:, g * 128:(g + 1) * 128] for g in range(G)]
                for s in (16, 8, 4):
                    m = (lane & s) == 0
                    n = len(cur) // 2
                    cur = [jnp.where(m, cur[t], cur[t + n]) + swap(jnp.where(m, cur[t + n], cur[t]), s)
                           for t in range(n)]
                y = cur[0]
                for s in (2, 1):
                    y = y + swap(y, s)
                r = gh[half] * pltpu.reciprocal(y + 1e-6, approx=True)
                return [pq[half][g] * jnp.take_along_axis(r, (lane & 96) + 4 * g, axis=1) for g in range(G)]

            def hchunk(c0, c1):
                c11, c12, c21, c22 = up_quads(c0, c1)
                def act(gt, up, g_):
                    return gt * pltpu.reciprocal(1.0 + jnp.exp(-gt), approx=True) * (up * (1.0 - g_))
                return act(c11, c12, gh[0]), act(c21, c22, gh[1])

            for j in range(HF // fs):
                c0, c1 = j * fs, (j + 1) * fs
                a11, a21 = hchunk(c0, c1)
                a12, a22 = hchunk(HF + c0, HF + c1)
                for n, t_ in enumerate(_a_combos(a11, a12, a21, a22)):
                    ad_v[n, :, c0:c1] = t_.astype(BF)
                if j + 1 == norm_at:
                    pt, pb = vpu_norm(0), vpu_norm(1)
                    for u in range(G // 2):
                        for n, t_ in enumerate(_a_combos(pt[u], pt[u + 4], pb[u], pb[u + 4])):
                            ad_v[n, :, HF + u * 128:HF + (u + 1) * 128] = t_.astype(BF)
            for s in range(osplit // 2):
                c0, c1 = s * oc, (s + 1) * oc
                c11, c12, c21, c22 = _c_combos(lambda n: _dot(ad_v[n], bd_v[n, 0:KD, c0:c1]))
                for (ct, cb, off) in ((c11, c21, 0), (c12, c22, HD)):
                    o_v[pl.ds(rr, tm2), off + c0:off + c1] = jnp.concatenate([ct, cb], axis=0).astype(BF)
                    o_copy(rr, (off + c0) // oc).start()
            return carry
        with scope("phase2"):
            lax.fori_loop(0, n2, p2, 0)
        with scope("tail"):
            pltpu.make_async_copy(o_v, o_hbm, osem).wait()

    def fn(A_x, A_wqkv, A_wo, B_x, B_w1, B_w3, B_w2, gate_w):
        x = A_x.reshape(S, D)
        anyspec = pl.BlockSpec(memory_space=pl.ANY)
        out = pl.pallas_call(
            kernel,
            in_specs=[anyspec] * 7,
            out_specs=anyspec,
            out_shape=jax.ShapeDtypeStruct((S, D), BF),
            scratch_shapes=[
                pltpu.VMEM((S, D), BF),
                pltpu.VMEM((D, 2 * D), BF),
                pltpu.VMEM((D, D), BF),
                pltpu.VMEM((NC + 1, 7, HD, CW), BF),
                pltpu.VMEM((NC + 1, 2, HD, CW), BF),
                pltpu.VMEM((7, KD + CR, HD), BF),
                pltpu.VMEM((2, HF + CR, HD), BF),
                pltpu.VMEM((D,), BF),
                pltpu.VMEM((S, D), BF),
                pltpu.VMEM((D, D), F32),
                pltpu.VMEM((8, D), F32),
                pltpu.VMEM((7, hm, KD), BF),
                pltpu.VMEM((1, D), F32),
                pltpu.VMEM((16, 128), jnp.int32),
                pltpu.VMEM((7, HD, HD), BF),
                pltpu.SemaphoreType.DMA((nsem,)),
            ],
            compiler_params=pltpu.CompilerParams(vmem_limit_bytes=vmem_mb * 1024 * 1024),
        )(x, A_wqkv, A_wo, B_w1, B_w3, B_w2, gate_w)
        return out.reshape(1, S, D)
    return fn


_impl = make(cr=288, mfa=0.75)


@jax.jit
def pallas_gated_mix__linear_attn_block__glu_gated_swiglu__prompt_kernel(
    A_x: jax.Array,
    A_wqkv: jax.Array,
    A_wo: jax.Array,
    B_x: jax.Array,
    B_w1: jax.Array,
    B_w3: jax.Array,
    B_w2: jax.Array,
    gate_w: jax.Array,
):
    return _impl(A_x, A_wqkv, A_wo, B_x, B_w1, B_w3, B_w2, gate_w)
```

```python
import jax
import jax.numpy as jnp
from jax import lax
from jax.experimental import pallas as pl
from jax.experimental.pallas import tpu as pltpu

BF = jnp.bfloat16
F32 = jnp.float32

S, D, F, H = 2048, 1024, 3584, 32
DH = D // H
G = D // 128
HD, HF = D // 2, F // 2
WU = F + HD
KD = HF + HD

R0 = 128
TM1 = 384
N1 = (S - R0) // TM1
TM2 = 256
N2 = S // TM2
HM = TM2 // 2
KCOLS = ((0, 256), (512, 768), (256, 512), (768, 1024))
NC = N1 - 1
CW = WU // NC
PW = CW // 2
CR = 288
CM = HF - NC * CR
CMA = CM * 3 // 4 // 16 * 16
FS = 256
OC = 256
RAW = (1, 4)
NSEM = 1 + len(KCOLS) + N1 + NC + 3

assert R0 + N1 * TM1 == S and NC * CW == WU and F % PW == 0 and CW % FS == 0 and HF % FS == 0


def _phi(t):
    return jnp.where(t > 0, t + 1.0, jnp.exp(t)) + 1e-6


def _dot(a, b):
    return jnp.dot(a, b, preferred_element_type=F32)


def _a_combos(a11, a12, a21, a22):
    return [a11 + a22, a21 + a22, a11, a22, a11 + a12, a21 - a11, a12 - a22]


def _b_combos(b11, b12, b21, b22):
    return [b11 + b22, b11, b12 - b22, b21 - b11, b22, b11 + b12, b21 + b22]


def _c_combos(prod):
    m = {n: prod(n) for n in (0, 3, 4, 6, 1, 2, 5)}
    return (m[0] + m[3] - m[4] + m[6], m[2] + m[4], m[1] + m[3], m[0] - m[1] + m[2] + m[5])


def _w_sums(b11, b12, b21, b22, tie):
    f = [t.astype(F32) for t in (b11, b12, b21, b22)]
    f[0] = f[0] + tie
    f[3] = f[3] + tie
    return {n: t.astype(BF) for n, t in enumerate(_b_combos(*f)) if n not in RAW}


def _tie(v, zero):
    return lax.bitcast_convert_type(lax.bitcast_convert_type(v, jnp.int32) & zero, F32)


def _kernel(x_hbm, wqkv_hbm, wo_hbm, w1_hbm, w3_hbm, w2_hbm, gw_hbm, o_hbm,
            x_v, wkv_v, wo_v, bu_v, su_v, bd_v, sd_v, gw_v, o_v, kx_acc, z_acc, ad_v, zr_v, zero_v, bk_v, sems):
    xbase = 1 + len(KCOLS)
    wbase = xbase + N1
    rsem, osem, lsem = (sems.at[wbase + NC + t] for t in range(3))

    cx0 = pltpu.make_async_copy(x_hbm.at[pl.ds(0, R0)], x_v.at[pl.ds(0, R0)], sems.at[0])
    ck = [pltpu.make_async_copy(wqkv_hbm.at[:, pl.ds(D + a, b - a)], wkv_v.at[:, pl.ds(a, b - a)], sems.at[1 + c])
          for c, (a, b) in enumerate(KCOLS)]

    def x_copy(i):
        rr = R0 + i * TM1
        if not isinstance(i, int):
            rr = pl.multiple_of(rr, 16)
        return pltpu.make_async_copy(x_hbm.at[pl.ds(rr, TM1)], x_v.at[pl.ds(rr, TM1)], sems.at[xbase + i])

    def d_copies(lo, n, sem):
        return [pltpu.make_async_copy(w2_hbm.at[pl.ds(r + lo, n), pl.ds(c, HD)], dst.at[slot, pl.ds(lo, n), :], sem)
                for (dst, slot, r, c) in ((bd_v, 1, 0, 0), (sd_v, 1, HF, 0), (sd_v, 0, 0, HD), (bd_v, 4, HF, HD))]

    def w_copies(c):
        static = isinstance(c, int)
        sem = sems.at[wbase + c]
        out = []
        for p in range(CW // PW):
            col = c * CW + p * PW
            for (dst, slot, left, r) in ((bu_v, 1, True, 0), (su_v, 1, True, HD), (su_v, 0, False, 0), (bu_v, 4, False, HD)):
                if static and col >= F:
                    src = wqkv_hbm.at[pl.ds(r, HD), pl.ds(col - F + (0 if left else HD), PW)]
                else:
                    src = (w1_hbm if left else w3_hbm).at[pl.ds(r, HD), pl.ds(col if static else pl.multiple_of(col, PW), PW)]
                out.append(pltpu.make_async_copy(src, dst.at[c, slot, :, pl.ds(p * PW, PW)], sem))
        return out + d_copies(c * CR if static else pl.multiple_of(c * CR, 16), CR, sem)

    crest = [pltpu.make_async_copy(gw_hbm, gw_v, rsem),
             pltpu.make_async_copy(wqkv_hbm.at[:, pl.ds(2 * D, D)], wkv_v.at[:, pl.ds(D, D)], rsem),
             pltpu.make_async_copy(wo_hbm, wo_v, rsem)] + d_copies(NC * CR, CMA, rsem)
    clast = d_copies(NC * CR + CMA, CM - CMA, lsem)
    order = [cx0] + ck + [x_copy(0)]
    for c in range(NC):
        order += [x_copy(c + 1)] + w_copies(c)
    for c in order + crest + clast:
        c.start()

    zero_v[...] = jnp.zeros((16, 128), jnp.int32)

    def kx_of(pkb, xi):
        return lax.dot_general(pkb, xi, (((0,), (0,)), ((), ())), preferred_element_type=F32)

    zero0 = zero_v[...]

    def wk_sums(lo, hi, val):
        todo = [(r, c) for c in range(lo, hi, 128) for r in range(0, HD, 16)]
        tiles = [(r, c) for c in range(0, val.shape[1], 128) for r in range(0, val.shape[0], 16)]
        tiles = tiles[:max(1, len(tiles) * 6 // 8)]
        per = -(-len(todo) // len(tiles))
        for (r1, c1) in tiles:
            part, todo = todo[:per], todo[per:]
            if part:
                tie = _tie(val[r1:r1 + 16, c1:c1 + 128], zero0)
            for (q, d) in part:
                r, r2, cs, cs2 = slice(q, q + 16), slice(HD + q, HD + q + 16), slice(d, d + 128), slice(HD + d, HD + d + 128)
                for n, t in _w_sums(wkv_v[r, cs], wkv_v[r, cs2], wkv_v[r2, cs], wkv_v[r2, cs2], tie).items():
                    bk_v[n, r, cs] = t
        assert not todo

    prev = None
    for c, (a, b) in enumerate(KCOLS):
        if c == 0:
            cx0.wait()
        ck[c].wait()
        xi = x_v[0:R0, :]
        pk = _phi(_dot(xi, wkv_v[:, a:b]))
        z_acc[:, a:b] = jnp.sum(pk.reshape(R0 // 8, 8, b - a), axis=0)
        if c == 1:
            wk_sums(a - HD, b - HD, pk)
        if prev is not None:
            kx_acc[prev[1]:prev[2], :] = kx_of(prev[0], xi)
        prev = (pk.astype(BF), a, b)
    kx = kx_of(prev[0], xi)
    kx_acc[prev[1]:prev[2], :] = kx
    wk_sums(prev[1] - HD, prev[2] - HD, kx)

    def p1(i, carry):
        x_copy(i).wait()

        @pl.when(jnp.logical_and(i > 0, i < NC))
        def _():
            for c in w_copies(i - 1):
                c.wait()

        @pl.when(i == NC)
        def _():
            for c in w_copies(NC - 1):
                c.wait()

        cc = jnp.where(i == 0, NC, i - 1)
        ro = pl.multiple_of(jnp.where(i == 0, KD, (i - 1) * CR), 16)
        so = pl.multiple_of(jnp.where(i == 0, HF, (i - 1) * CR), 16)
        xi = x_v[pl.ds(pl.multiple_of(R0 + i * TM1, 16), TM1), :]
        todo = [(True, r, c) for r in range(0, HD, 16) for c in range(0, CW, 128)]
        todo += [(False, r, c) for r in range(0, CR, 16) for c in range(0, HD, 128)]
        zero = zero_v[...]
        state = [0, 0.0]

        def tile(up, r1, c1, tie):
            cs = slice(c1, c1 + 128)
            if up:
                r = slice(r1, r1 + 16)
                for n, t in _w_sums(bu_v[cc, 1, r, cs], su_v[cc, 0, r, cs], su_v[cc, 1, r, cs], bu_v[cc, 4, r, cs], tie).items():
                    bu_v[cc, n, r, cs] = t
            else:
                r, q = pl.ds(ro + r1, 16), pl.ds(so + r1, 16)
                for n, t in _w_sums(bd_v[1, r, cs], sd_v[0, q, cs], sd_v[1, q, cs], bd_v[4, r, cs], tie).items():
                    bd_v[n, r, cs] = t

        def paced(val, share):
            tiles = [(r, c) for c in range(0, val.shape[1], 128) for r in range(0, val.shape[0], 16)]
            for k, (r1, c1) in enumerate(tiles):
                goal = int(round((state[1] + share * min(1.0, (k + 1) / (len(tiles) * 0.85))) * len(todo)))
                if goal > state[0]:
                    tie = _tie(val[r1:r1 + 16, c1:c1 + 128], zero)
                    while state[0] < goal:
                        tile(*todo[state[0]], tie)
                        state[0] += 1
            state[1] += share

        hr = TM1 // 2
        xf = xi.astype(F32)
        xa = [t.astype(BF) for t in _a_combos(xf[0:hr, 0:HD], xf[0:hr, HD:D], xf[hr:TM1, 0:HD], xf[hr:TM1, HD:D])]

        def bk(n, c0, c1):
            if n == 1:
                return wkv_v[0:HD, c0:c1]
            if n == 4:
                return wkv_v[HD:D, HD + c0:HD + c1]
            return bk_v[n, :, c0:c1]

        kshare, kc = 0.15, 256
        pkq = [[], [], [], []]
        for c0 in range(0, HD, kc):
            quads = _c_combos(lambda n: _dot(xa[n], bk(n, c0, c0 + kc)))
            for q in range(4):
                pkq[q].append(_phi(quads[q]))
            for side in range(2):
                zs = pkq[side][-1] + pkq[2 + side][-1]
                z_acc[:, side * HD + c0:side * HD + c0 + kc] += jnp.sum(zs.reshape(hr // 8, 8, kc), axis=0)
            paced(pkq[3][-1], kshare * kc / HD)
        pq_ = [jnp.concatenate(p, axis=1) for p in pkq]
        pkb = jnp.concatenate([jnp.concatenate([pq_[0], pq_[1]], axis=1),
                               jnp.concatenate([pq_[2], pq_[3]], axis=1)], axis=0).astype(BF)
        kx = kx_of(pkb, xi)
        kx_acc[...] += kx
        paced(kx, 1.0 - kshare)
        assert state[0] == len(todo)
        return carry

    lax.fori_loop(0, N1, p1, 0)

    for c in crest:
        c.wait()
    same = (lax.broadcasted_iota(jnp.int32, (128, 128), 0) // DH
            == lax.broadcasted_iota(jnp.int32, (128, 128), 1) // DH)
    zr_v[...] = jnp.sum(z_acc[...], axis=0, keepdims=True)
    kvf = [_dot(kx_acc[g * 128:(g + 1) * 128, :].astype(BF), wkv_v[:, D + g * 128:D + (g + 1) * 128]) for g in range(G)]
    kvs = [jnp.where(same, t, 0.0).astype(BF) for t in kvf]
    todo2 = [(r, c) for r in range(NC * CR, HF, 16) for c in range(0, HD, 128)]
    done2 = [0]
    zero2 = zero_v[...]

    def paced2(val, frac):
        goal = int(round(frac * len(todo2)))
        if goal > done2[0]:
            tie = _tie(val, zero2)
            while done2[0] < goal:
                r1, c1 = todo2[done2[0]]
                r, cs = slice(r1, r1 + 16), slice(c1, c1 + 128)
                for n, t in _w_sums(bd_v[1, r, cs], sd_v[0, r, cs], sd_v[1, r, cs], bd_v[4, r, cs], tie).items():
                    bd_v[n, r, cs] = t
                done2[0] += 1

    fa = CMA / CM
    for g in range(G):
        for u in range(8):
            paced2(kvf[g][u * 16:(u + 1) * 16, :], fa * (g * 8 + u + 1) / 64.0)
    assert done2[0] * 16 <= CMA * (HD // 128)
    for c in clast:
        c.wait()
    for g in range(G // 2):
        mt = _dot(kvs[g], wo_v[g * 128:(g + 1) * 128, :])
        mb = _dot(kvs[g + 4], wo_v[(g + 4) * 128:(g + 5) * 128, :])
        for n, t in enumerate(_b_combos(mt[:, 0:HD], mt[:, HD:D], mb[:, 0:HD], mb[:, HD:D])):
            bd_v[n, HF + g * 128:HF + (g + 1) * 128, :] = t.astype(BF)
        for w, mm in enumerate((mt, mb)):
            for u in range(8):
                for v in range(0, 128, 64):
                    k = ((g * 2 + w) * 8 + u) * 2 + v // 64 + 1
                    paced2(mm[v:v + 16, u * 128:(u + 1) * 128], min(1.0, fa + (1 - fa) * k / (128.0 * 0.85)))
    assert done2[0] == len(todo2)

    def p2(i, carry):
        rr = pl.multiple_of(i * TM2, TM2)
        xf = x_v[pl.ds(rr, TM2), :].astype(F32)
        gate = jax.nn.sigmoid(jnp.sum(xf * gw_v[...].astype(F32).reshape(1, D), axis=-1, keepdims=True))
        au = [t.astype(BF) for t in _a_combos(xf[0:HM, 0:HD], xf[0:HM, HD:D], xf[HM:TM2, 0:HD], xf[HM:TM2, HD:D])]
        gh = (gate[0:HM], gate[HM:TM2])

        def up_quads(c0):
            return _c_combos(lambda n: _dot(au[n], bu_v[c0 // CW, n, :, c0 % CW:c0 % CW + FS]))

        pq = [[None] * G, [None] * G]
        for c0 in range(0, HD, FS):
            quads = up_quads(F + c0)
            for half in range(2):
                for side in range(2):
                    t = _phi(quads[2 * half + side])
                    for u in range(FS // 128):
                        pq[half][(side * HD + c0) // 128 + u] = t[:, u * 128:(u + 1) * 128]

        def normalised_q(half):
            lane = lax.broadcasted_iota(jnp.int32, (HM, 128), 1)
            zrow = zr_v[...]

            def swap(y, s):
                return jnp.take_along_axis(y, lane ^ s, axis=1)

            cur = [pq[half][g] * zrow[:, g * 128:(g + 1) * 128] for g in range(G)]
            for s in (16, 8, 4):
                m = (lane & s) == 0
                n = len(cur) // 2
                cur = [jnp.where(m, cur[t], cur[t + n]) + swap(jnp.where(m, cur[t + n], cur[t]), s) for t in range(n)]
            y = cur[0]
            for s in (2, 1):
                y = y + swap(y, s)
            r = gh[half] * pltpu.reciprocal(y + 1e-6, approx=True)
            return [pq[half][g] * jnp.take_along_axis(r, (lane & 96) + 4 * g, axis=1) for g in range(G)]

        def h_halves(c0):
            c11, c12, c21, c22 = up_quads(c0)

            def act(gt, up, g):
                return gt * pltpu.reciprocal(1.0 + jnp.exp(-gt), approx=True) * (up * (1.0 - g))

            return act(c11, c12, gh[0]), act(c21, c22, gh[1])

        for j in range(HF // FS):
            c0 = j * FS
            a11, a21 = h_halves(c0)
            a12, a22 = h_halves(HF + c0)
            for n, t in enumerate(_a_combos(a11, a12, a21, a22)):
                ad_v[n, :, c0:c0 + FS] = t.astype(BF)
            if j == 0:
                qt, qb = normalised_q(0), normalised_q(1)
                for u in range(G // 2):
                    for n, t in enumerate(_a_combos(qt[u], qt[u + 4], qb[u], qb[u + 4])):
                        ad_v[n, :, HF + u * 128:HF + (u + 1) * 128] = t.astype(BF)

        for c0 in range(0, HD, OC):
            c11, c12, c21, c22 = _c_combos(lambda n: _dot(ad_v[n], bd_v[n, 0:KD, c0:c0 + OC]))
            for (ct, cb, off) in ((c11, c21, c0), (c12, c22, HD + c0)):
                o_v[pl.ds(rr, TM2), off:off + OC] = jnp.concatenate([ct, cb], axis=0).astype(BF)
                pltpu.make_async_copy(o_v.at[pl.ds(rr, TM2), pl.ds(off, OC)],
                                      o_hbm.at[pl.ds(rr, TM2), pl.ds(off, OC)], osem).start()
        return carry

    lax.fori_loop(0, N2, p2, 0)
    pltpu.make_async_copy(o_v, o_hbm, osem).wait()


@jax.jit
def pallas_gated_mix__linear_attn_block__glu_gated_swiglu__prompt_kernel(
    A_x: jax.Array,
    A_wqkv: jax.Array,
    A_wo: jax.Array,
    B_x: jax.Array,
    B_w1: jax.Array,
    B_w3: jax.Array,
    B_w2: jax.Array,
    gate_w: jax.Array,
):
    del B_x
    hbm = pl.BlockSpec(memory_space=pl.ANY)
    out = pl.pallas_call(
        _kernel,
        in_specs=[hbm] * 7,
        out_specs=hbm,
        out_shape=jax.ShapeDtypeStruct((S, D), BF),
        scratch_shapes=[
            pltpu.VMEM((S, D), BF),
            pltpu.VMEM((D, 2 * D), BF),
            pltpu.VMEM((D, D), BF),
            pltpu.VMEM((NC + 1, 7, HD, CW), BF),
            pltpu.VMEM((NC + 1, 2, HD, CW), BF),
            pltpu.VMEM((7, KD + CR, HD), BF),
            pltpu.VMEM((2, HF + CR, HD), BF),
            pltpu.VMEM((D,), BF),
            pltpu.VMEM((S, D), BF),
            pltpu.VMEM((D, D), F32),
            pltpu.VMEM((8, D), F32),
            pltpu.VMEM((7, HM, KD), BF),
            pltpu.VMEM((1, D), F32),
            pltpu.VMEM((16, 128), jnp.int32),
            pltpu.VMEM((7, HD, HD), BF),
            pltpu.SemaphoreType.DMA((NSEM,)),
        ],
        compiler_params=pltpu.CompilerParams(vmem_limit_bytes=120 * 1024 * 1024),
    )(A_x.reshape(S, D), A_wqkv, A_wo, B_w1, B_w3, B_w2, gate_w)
    return out.reshape(1, S, D)
```
